```python
import jax
import jax.numpy as jnp

def _softmax(x, axis=-1):
    return jax.nn.softmax(x, axis=axis)

def _gelu(x):
    return jax.nn.gelu(x, approximate=True)

def _silu(x):
    return jax.nn.silu(x)

def _sigmoid(x):
    return jax.nn.sigmoid(x)

def _layernorm(x, axis=-1, eps=1e-05):
    m = jnp.mean(x, axis=axis, keepdims=True)
    v = jnp.var(x, axis=axis, keepdims=True)
    return (x - m) / jnp.sqrt(v + eps)

def _scatter_add(tgt, idx, src, axis=0):
    return tgt.at[idx].add(src)

def _segment_sum(src, seg, n):
    return jax.ops.segment_sum(src, seg, n)

class _Rng:

    def __init__(self, key):
        self._k = key

    def _next(self):
        self._k, sub = jax.random.split(self._k)
        return sub

    def normal(self, shape):
        return jax.random.normal(self._next(), shape, dtype=jnp.bfloat16)

    def randint(self, lo, hi, shape):
        return jax.random.randint(self._next(), shape, lo, hi, dtype=jnp.int32)

    def uniform(self, shape, lo=0.0, hi=1.0):
        return jax.random.uniform(self._next(), shape, jnp.bfloat16, lo, hi)

    def permutation(self, n):
        return jax.random.permutation(self._next(), n)
kernel_name = 'adaLN_cond__ssm_conv_h3__glu_gated_bilinear__prompt'

def setup_inputs():
    _rng = _Rng(jax.random.key(int.from_bytes(__import__("os").urandom(4), "little")))
    _w = lambda a: (lambda t: t.astype(jnp.bfloat16) if jnp.issubdtype(t.dtype, jnp.floating) else t)(jnp.asarray(a))

    def _A_setup():
        B, S, D = (1, 2048, 640)
        ks = 4
        return {'q': _w((lambda *s: _rng.normal(s) * 0.05)(B, S, D)), 'k': _w((lambda *s: _rng.normal(s) * 0.05)(B, S, D)), 'v': _w((lambda *s: _rng.normal(s) * 0.05)(B, S, D)), 'shift_k': _w((lambda *s: _rng.normal(s) * 0.05)(D, ks) * 0.5), 'ssm_k': _w((lambda *s: _rng.normal(s) * 0.05)(D, S) * (1.0 / S ** 0.5)), 'ssm_D': _w((lambda *s: _rng.normal(s) * 0.05)(D))}
    _A_in = _A_setup()

    def _B_setup():
        B, S, D, F = (1, 2048, 640, 1536)
        return {'x': _w((lambda *s: _rng.normal(s) * 0.05)(B, S, D)), 'w_gate': _w((lambda *s: _rng.normal(s) * 0.05)(D, F) * D ** (-0.5)), 'w_up': _w((lambda *s: _rng.normal(s) * 0.05)(D, F) * D ** (-0.5)), 'w_down': _w((lambda *s: _rng.normal(s) * 0.05)(F, D) * F ** (-0.5))}
    _B_in = _B_setup()
    return {'A_q': _A_in['q'], 'A_k': _A_in['k'], 'A_v': _A_in['v'], 'A_shift_k': _A_in['shift_k'], 'A_ssm_k': _A_in['ssm_k'], 'A_ssm_D': _A_in['ssm_D'], 'B_x': _B_in['x'], 'B_w_gate': _B_in['w_gate'], 'B_w_up': _B_in['w_up'], 'B_w_down': _B_in['w_down'], 'c': _w((lambda *s: _rng.normal(s) * 0.05)(1, 640)), 'w_mod': _w((lambda *s: _rng.normal(s) * 0.05)(640, 6 * 640) * 640 ** (-0.5))}

def reference(A_q, A_k, A_v, A_shift_k, A_ssm_k, A_ssm_D, B_x, B_w_gate, B_w_up, B_w_down, c, w_mod):

    def _A_ref(q, k, v, shift_k, ssm_k, ssm_D):
        B, S, D = q.shape
        ks = shift_k.shape[-1]
        k_pad = jnp.pad(k, ((0, 0), (ks - 1, 0), (0, 0)))
        k_shift = jnp.zeros_like(k)
        for t in range(ks):
            k_shift = k_shift + k_pad[:, t:t + S, :] * shift_k[:, ks - 1 - t][None, None, :]
        kv = k_shift * v
        L = 2 * S
        kv_pad = jnp.pad(kv, ((0, 0), (0, S), (0, 0)))
        kf_pad = jnp.pad(ssm_k, ((0, 0), (0, S)))
        kv_f = (lambda x, axes=(-2, -1): jnp.fft.rfft2(x.astype(jnp.float32), axes=axes))(kv_pad[:, None, :, :], axes=(1, 2))
        kf_f = (lambda x, axes=(-2, -1): jnp.fft.rfft2(x.astype(jnp.float32), axes=axes))(kf_pad[:, None, :], axes=(1, 2))
        kf_f = (lambda x, *d: x.transpose(*d))(kf_f, 1, 2, 0)
        y_f = kv_f * kf_f[None, :, :, :]
        y = (lambda x, s, axes=(-2, -1): jnp.fft.irfft2(x, s=s, axes=axes).astype(jnp.bfloat16))(y_f, (1, L), axes=(1, 2))[:, 0, :S, :]
        y = y + kv * ssm_D[None, None, :]
        return q * y

    def _B_ref(x, w_gate, w_up, w_down):
        g = jnp.einsum('bsd,df->bsf', x, w_gate)
        u = jnp.einsum('bsd,df->bsf', x, w_up)
        h = g * u
        return jnp.einsum('bsf,fd->bsd', h, w_down)
    x = A_q
    mod = (_silu(c) @ w_mod).reshape(c.shape[0], 6, 1, -1)
    sa, ca, ga, sb, cb, gb = (mod[:, 0].copy(), mod[:, 1].copy(), mod[:, 2].copy(), mod[:, 3].copy(), mod[:, 4].copy(), mod[:, 5].copy())
    h = _layernorm(x, axis=-1) * (1 + ca) + sa
    x = x + ga * _A_ref(h, A_k, A_v, A_shift_k, A_ssm_k, A_ssm_D)
    h = _layernorm(x, axis=-1) * (1 + cb) + sb
    x = x + gb * _B_ref(h, B_w_gate, B_w_up, B_w_down)
    return x
```

```python
import numpy as np

import jax
import jax.numpy as jnp
import jax.experimental.pallas as pl
import jax.experimental.pallas.tpu as pltpu

S, D, FF = 2048, 640, 1536
C = 128
BM = 256
NSTEP = S // BM
HALO = 16
EPS = 1e-5

KB, UB, YB = 0, 16, 32
NSLOT = 48

FC = 512
NF = FF // FC
ROWS = 8

F32, BF16 = jnp.float32, jnp.bfloat16
FLAGS = None

V_A1, V_SA, V_GA, V_B1, V_SB, V_GB, V_W0, V_D, V_SGN = 0, 1, 2, 3, 4, 5, 6, 10, 11


def _dft_matrices():
    f = np.arange(C, dtype=np.float64)[None, :, None] + 0.5
    s = np.arange(4 * C, dtype=np.float64).reshape(4, 1, C)
    ang = 2.0 * np.pi * f * s / (2 * C)
    fwd = np.concatenate([np.cos(ang), -np.sin(ang)], axis=1)
    inv = np.swapaxes(fwd, 1, 2) / C
    return fwd.astype(np.float32).astype(BF16), inv.astype(np.float32).astype(BF16)


_SCHED = [
    [(2, 1), (3, 2), (4, 3), (5, 4), (6, 3), (7, 1), (7, 4)],
    [(3, 1), (4, 2), (5, 2), (6, 1), (6, 4), (7, 2), (7, 5)],
    [(4, 1), (5, 1), (5, 3), (6, 2), (6, 5), (7, 3), (7, 6)],
]


def _pack(vals):
    r = 0
    for t, x in enumerate(vals):
        r |= x << (3 * (t + 1))
    return r


def _layernorm(x):
    m = jnp.mean(x, axis=1, keepdims=True)
    xc = x - m
    v = jnp.mean(xc * xc, axis=1, keepdims=True)
    return xc * jax.lax.rsqrt(v + EPS)


def _kernel(q_hbm, k_hbm, v_hbm, sh_hbm, ssm_hbm, d_hbm, wg_hbm, wu_hbm, wd_hbm, c_hbm, wm_hbm,
            f_hbm, g_hbm, o_hbm,
            q_s, k_s, v_s, sh_s, ssm_s, d_s, wg_s, wu_s, wd_s, c_s, wm_s, f_s, g_s,
            pool, vec, kv_s, x1_s, h2_s, a_s, out_s,
            sem_small, sem_ssm, sem_wm, sem_k, sem_v, sem_q, sem_wg, sem_wu, sem_wd, sem_o):

    def cp_small(i):
        src, dst = [(c_hbm, c_s), (sh_hbm, sh_s), (d_hbm, d_s), (f_hbm, f_s), (g_hbm, g_s)][i]
        return pltpu.make_async_copy(src, dst, sem_small.at[i])

    NSP = 4
    SP = S // NSP

    def cp_ssm(p):
        return pltpu.make_async_copy(ssm_hbm.at[:, pl.ds(p * SP, SP)], ssm_s.at[:, pl.ds(p * SP, SP)], sem_ssm.at[p])

    def cp_wm(s):
        return pltpu.make_async_copy(wm_hbm.at[:, pl.ds(s * D, D)], wm_s.at[s], sem_wm.at[s])

    def cp_k(t):
        return pltpu.make_async_copy(k_hbm.at[pl.ds(t * BM, BM)], k_s.at[pl.ds(HALO + t * BM, BM)], sem_k.at[t])

    def cp_v(t):
        return pltpu.make_async_copy(v_hbm.at[pl.ds(t * BM, BM)], v_s.at[pl.ds(t * BM, BM)], sem_v.at[t])

    def cp_q(t):
        return pltpu.make_async_copy(q_hbm.at[pl.ds(t * BM, BM)], q_s.at[pl.ds(t * BM, BM)], sem_q.at[t])

    def cp_wg(j):
        return pltpu.make_async_copy(wg_hbm.at[:, pl.ds(j * FC, FC)], wg_s.at[j], sem_wg.at[j])

    def cp_wu(j):
        return pltpu.make_async_copy(wu_hbm.at[:, pl.ds(j * FC, FC)], wu_s.at[j], sem_wu.at[j])

    def cp_wd(j):
        return pltpu.make_async_copy(wd_hbm.at[pl.ds(j * FC, FC)], wd_s.at[pl.ds(j * FC, FC)], sem_wd.at[j])

    def cp_o(t):
        return pltpu.make_async_copy(out_s.at[pl.ds(t * BM, BM)], o_hbm.at[pl.ds(t * BM, BM)], sem_o.at[t])

    for i in range(5):
        cp_small(i).start()
    for p in range(NSP):
        cp_ssm(p).start()

    def vrow(i):
        return vec[i]

    def bc(i, rows):
        return jnp.broadcast_to(vec[i, 0:1, :], (rows, D))

    def conv_fwd(t):
        R = 64
        for r in range(0, BM, R):
            kk = k_s[pl.ds(pl.multiple_of(t * BM + r, HALO), R + HALO), :].astype(F32)
            ks = kk[HALO:] * bc(V_W0, R)
            for j in range(1, 4):
                ks = ks + kk[HALO - j:HALO - j + R] * bc(V_W0 + j, R)
            vv = v_s[pl.ds(pl.multiple_of(t * BM + r, R), R), :].astype(F32)
            kv_s[r:r + R, :] = (ks * vv).astype(BF16)
        for c in range(2):
            u = jnp.dot(f_s[2 * (t % 2) + c], kv_s[c * C:(c + 1) * C, :], preferred_element_type=F32)
            pool[UB + 2 * t + c] = u

    def cmul(kr, ki, ur, ui):
        return kr * ur - ki * ui, kr * ui + ki * ur

    def block(I, J, L, diag, first):
        ys, us, ks = YB + 2 * I, UB + 2 * J, KB + 2 * L
        for r in range(0, C, ROWS):
            re, im = slice(r, r + ROWS), slice(C + r, C + r + ROWS)
            u0r, u0i = pool[us, re, :], pool[us, im, :]
            u1r, u1i = pool[us + 1, re, :], pool[us + 1, im, :]
            kbr, kbi = pool[ks, re, :], pool[ks, im, :]
            kcr, kci = pool[ks + 1, re, :], pool[ks + 1, im, :]
            ar, ai = cmul(kbr, kbi, u0r, u0i)
            if not diag:
                kar, kai = pool[ks - 1, re, :], pool[ks - 1, im, :]
                cr, ci = cmul(kar, kai, u1r, u1i)
                ar, ai = ar + cr, ai + ci
            br, bi = cmul(kcr, kci, u0r, u0i)
            dr, di = cmul(kbr, kbi, u1r, u1i)
            br, bi = br + dr, bi + di
            if not first:
                ar, ai = pool[ys, re, :] + ar, pool[ys, im, :] + ai
                br, bi = pool[ys + 1, re, :] + br, pool[ys + 1, im, :] + bi
            pool[ys, re, :] = ar
            pool[ys, im, :] = ai
            pool[ys + 1, re, :] = br
            pool[ys + 1, im, :] = bi

    def inverse_post(t, first=False):
        slot = t % 2
        for c in range(2):
            if first and c == 0:
                yf = pool[YB].astype(BF16)
            else:
                yf = (pool[YB + 2 * t + c] + pool[YB + 2 * t + c - 1]).astype(BF16)
            y = jnp.dot(g_s[2 * (t % 2) + c], yf, preferred_element_type=F32)
            R = 64
            for r in range(0, C, R):
                rr = c * C + r
                kv = kv_s[rr:rr + R, :].astype(F32)
                yy = y[r:r + R] + kv * bc(V_D, R)
                x = q_s[pl.ds(pl.multiple_of(t * BM + rr, R), R), :].astype(F32)
                h1 = _layernorm(x) * bc(V_A1, R) + bc(V_SA, R)
                x1 = x + bc(V_GA, R) * (h1 * yy)
                x1_s[slot, rr:rr + R, :] = x1
                h2 = _layernorm(x1) * bc(V_B1, R) + bc(V_SB, R)
                h2_s[rr:rr + R, :] = h2.astype(BF16)

    def gate_up(j):
        h = h2_s[...]
        g = jnp.dot(h, wg_s[j], preferred_element_type=F32)
        u = jnp.dot(h, wu_s[j], preferred_element_type=F32)
        a_s[:, j * FC:(j + 1) * FC] = (g * u).astype(BF16)

    def down_out(t):
        slot = t % 2
        o = jnp.dot(a_s[...], wd_s[...], preferred_element_type=F32)
        o = x1_s[slot] + bc(V_GB, BM) * o
        out_s[pl.ds(pl.multiple_of(t * BM, BM), BM), :] = o.astype(BF16)

    k_s[0:HALO, :] = jnp.zeros((HALO, D), BF16)
    for i in range(5):
        cp_small(i).wait()
    sh = sh_s[...].astype(F32)
    for j in range(4):
        vec[V_W0 + j] = jnp.broadcast_to(sh[j:j + 1, :], (8, D))
    vec[V_D] = jnp.broadcast_to(d_s[...].astype(F32).reshape(1, D), (8, D))
    cf = c_s[...].astype(F32)
    sc = (cf * jax.nn.sigmoid(cf)).astype(BF16)
    sc = jnp.broadcast_to(sc, (16, D))

    def k_body(m, carry):
        chunk = ssm_s[:, pl.ds(pl.multiple_of(m * C, C), C)]
        pool[KB + m] = jax.lax.dot_general(f_s[m % 4], chunk, (((1,), (1,)), ((), ())),
                                           preferred_element_type=F32)
        return carry

    for p in range(NSP):
        cp_ssm(p).wait()
        if p == 1:
            cp_k(0).start(); cp_v(0).start()
            for s_ in range(3):
                cp_wm(s_).start()
        if p == 3:
            for s_ in range(3, 6):
                cp_wm(s_).start()
            cp_q(0).start(); cp_k(1).start(); cp_v(1).start()
        jax.lax.fori_loop(p * (SP // C), (p + 1) * (SP // C), k_body, 0)

    cp_k(0).wait()
    cp_v(0).wait()
    conv_fwd(0)
    for j in range(NF):
        cp_wg(j).start(); cp_wu(j).start()
    block(0, 0, 0, True, True)

    def b_body(I, carry):
        block(I, 0, I, False, True)
        return carry

    jax.lax.fori_loop(1, NSTEP, b_body, 0)

    def mod(s, dst, plus_one):
        cp_wm(s).wait()
        m = jnp.dot(sc, wm_s[s], preferred_element_type=F32)[0:8]
        m = m.astype(BF16).astype(F32)
        vec[dst] = 1.0 + m if plus_one else m

    cp_q(1).start()
    for j in range(NF):
        cp_wd(j).start()
    mod(0, V_SA, False)
    mod(1, V_A1, True)
    mod(2, V_GA, False)
    mod(3, V_SB, False)
    mod(4, V_B1, True)
    mod(5, V_GB, False)
    cp_q(0).wait()
    inverse_post(0, True)

    for j in range(NF):
        cp_wg(j).wait()
        cp_wu(j).wait()
        cp_wd(j).wait()

    def body(t, carry):
        cp_k(t).wait()
        cp_v(t).wait()
        cp_q(t).wait()
        @pl.when(t < NSTEP - 1)
        def _():
            cp_k(t + 1).start(); cp_v(t + 1).start(); cp_q(t + 1).start()
        conv_fwd(t)
        block(t, t, 0, True, False)
        for sched in _SCHED:
            I = (_pack([ij[0] for ij in sched]) >> (3 * t)) & 7
            J = (_pack([ij[1] for ij in sched]) >> (3 * t)) & 7
            block(I, J, I - J, False, False)
        for j in range(NF):
            gate_up(j)
        inverse_post(t)
        down_out(t - 1)
        cp_o(t - 1).start()
        return carry

    jax.lax.fori_loop(1, NSTEP, body, 0)

    for j in range(NF):
        gate_up(j)
    down_out(NSTEP - 1)
    cp_o(NSTEP - 1).start()
    for t in range(NSTEP):
        cp_o(t).wait()


@jax.jit
def pallas_adaLN_cond__ssm_conv_h3__glu_gated_bilinear__prompt_kernel(
    A_q: jax.Array,
    A_k: jax.Array,
    A_v: jax.Array,
    A_shift_k: jax.Array,
    A_ssm_k: jax.Array,
    A_ssm_D: jax.Array,
    B_x: jax.Array,
    B_w_gate: jax.Array,
    B_w_up: jax.Array,
    B_w_down: jax.Array,
    c: jax.Array,
    w_mod: jax.Array,
):
    del B_x
    fwd, inv = _dft_matrices()
    any_spec = pl.BlockSpec(memory_space=pl.ANY)
    scratch = [
        pltpu.VMEM((S, D), BF16),
        pltpu.VMEM((HALO + S, D), BF16),
        pltpu.VMEM((S, D), BF16),
        pltpu.VMEM((4, D), BF16),
        pltpu.VMEM((D, S), BF16),
        pltpu.VMEM((D,), BF16),
        pltpu.VMEM((NF, D, FC), BF16),
        pltpu.VMEM((NF, D, FC), BF16),
        pltpu.VMEM((FF, D), BF16),
        pltpu.VMEM((1, D), BF16),
        pltpu.VMEM((6, D, D), BF16),
        pltpu.VMEM((4, 2 * C, C), BF16),
        pltpu.VMEM((4, C, 2 * C), BF16),
        pltpu.VMEM((NSLOT, 2 * C, D), F32),
        pltpu.VMEM((12, 8, D), F32),
        pltpu.VMEM((BM, D), BF16),
        pltpu.VMEM((2, BM, D), F32),
        pltpu.VMEM((BM, D), BF16),
        pltpu.VMEM((BM, FF), BF16),
        pltpu.VMEM((S, D), BF16),
        pltpu.SemaphoreType.DMA((5,)),
        pltpu.SemaphoreType.DMA((4,)),
        pltpu.SemaphoreType.DMA((6,)),
        pltpu.SemaphoreType.DMA((NSTEP,)),
        pltpu.SemaphoreType.DMA((NSTEP,)),
        pltpu.SemaphoreType.DMA((NSTEP,)),
        pltpu.SemaphoreType.DMA((NF,)),
        pltpu.SemaphoreType.DMA((NF,)),
        pltpu.SemaphoreType.DMA((NF,)),
        pltpu.SemaphoreType.DMA((NSTEP,)),
    ]
    out = pl.pallas_call(
        _kernel,
        in_specs=[any_spec] * 13,
        out_specs=any_spec,
        out_shape=jax.ShapeDtypeStruct((S, D), BF16),
        scratch_shapes=scratch,
        compiler_params=pltpu.CompilerParams(vmem_limit_bytes=110 * 2**20, flags=FLAGS),
    )(A_q.reshape(S, D), A_k.reshape(S, D), A_v.reshape(S, D), A_shift_k.T, A_ssm_k, A_ssm_D,
      B_w_gate, B_w_up, B_w_down, c, w_mod, fwd, inv)
    return out.reshape(1, S, D)
```

```python
import numpy as np

import jax
import jax.numpy as jnp
import jax.experimental.pallas as pl
import jax.experimental.pallas.tpu as pltpu

S, D, FF = 2048, 640, 1536
C = 128
BM = 256
NSTEP = S // BM
HALO = 16
EPS = 1e-5

KB, UB, YB = 0, 16, 32
NSLOT = 48

FC = 512
NF = FF // FC
ROWS = 8

F32, BF16 = jnp.float32, jnp.bfloat16
FLAGS = None

V_A1, V_SA, V_GA, V_B1, V_SB, V_GB, V_W0, V_D, V_SGN = 0, 1, 2, 3, 4, 5, 6, 10, 11


def _dft_matrices():
    f = np.arange(C, dtype=np.float64)[None, :, None] + 0.5
    s = np.arange(4 * C, dtype=np.float64).reshape(4, 1, C)
    ang = 2.0 * np.pi * f * s / (2 * C)
    fwd = np.concatenate([np.cos(ang), -np.sin(ang)], axis=1)
    inv = np.swapaxes(fwd, 1, 2) / C
    return fwd.astype(np.float32).astype(BF16), inv.astype(np.float32).astype(BF16)


_SCHED = [
    [(3, 1), (4, 2), (5, 2), (6, 1), (6, 5), (7, 3)],
    [(3, 2), (4, 3), (5, 3), (6, 2), (7, 0), (7, 4)],
    [(4, 0), (5, 0), (5, 4), (6, 3), (7, 1), (7, 5)],
    [(4, 1), (5, 1), (6, 0), (6, 4), (7, 2), (7, 6)],
]
_ZERO_FROM = 4


def _pack(vals):
    r = 0
    for t, x in enumerate(vals):
        r |= x << (3 * (t + 2))
    return r


def _layernorm(x):
    m = jnp.mean(x, axis=1, keepdims=True)
    xc = x - m
    v = jnp.mean(xc * xc, axis=1, keepdims=True)
    return xc * jax.lax.rsqrt(v + EPS)


def _kernel(q_hbm, k_hbm, v_hbm, sh_hbm, ssm_hbm, d_hbm, wg_hbm, wu_hbm, wd_hbm, c_hbm, wm_hbm,
            f_hbm, g_hbm, o_hbm,
            q_s, k_s, v_s, sh_s, ssm_s, d_s, wg_s, wu_s, wd_s, c_s, wm_s, f_s, g_s,
            pool, vec, kv_s, x1_s, h2_s, a_s, out_s,
            sem_small, sem_ssm, sem_wm, sem_k, sem_v, sem_q, sem_wg, sem_wu, sem_wd, sem_o):

    def cp_small(i):
        src, dst = [(f_hbm, f_s), (sh_hbm, sh_s), (d_hbm, d_s), (c_hbm, c_s), (g_hbm, g_s)][i]
        return pltpu.make_async_copy(src, dst, sem_small.at[i])

    NSP = 4
    SP = S // NSP

    def cp_ssm(p):
        return pltpu.make_async_copy(ssm_hbm.at[:, pl.ds(p * SP, SP)], ssm_s.at[:, pl.ds(p * SP, SP)], sem_ssm.at[p])

    def cp_wm(s):
        return pltpu.make_async_copy(wm_hbm.at[:, pl.ds(s * D, D)], wm_s.at[s], sem_wm.at[s])

    def cp_k(t):
        return pltpu.make_async_copy(k_hbm.at[pl.ds(t * BM, BM)], k_s.at[pl.ds(HALO + t * BM, BM)], sem_k.at[t])

    def cp_v(t):
        return pltpu.make_async_copy(v_hbm.at[pl.ds(t * BM, BM)], v_s.at[pl.ds(t * BM, BM)], sem_v.at[t])

    def cp_q(t):
        return pltpu.make_async_copy(q_hbm.at[pl.ds(t * BM, BM)], q_s.at[pl.ds(t * BM, BM)], sem_q.at[t])

    def cp_wg(j):
        return pltpu.make_async_copy(wg_hbm.at[:, pl.ds(j * FC, FC)], wg_s.at[j], sem_wg.at[j])

    def cp_wu(j):
        return pltpu.make_async_copy(wu_hbm.at[:, pl.ds(j * FC, FC)], wu_s.at[j], sem_wu.at[j])

    def cp_wd(j):
        return pltpu.make_async_copy(wd_hbm.at[pl.ds(j * FC, FC)], wd_s.at[pl.ds(j * FC, FC)], sem_wd.at[j])

    def cp_o(t):
        return pltpu.make_async_copy(out_s.at[pl.ds(t * BM, BM)], o_hbm.at[pl.ds(t * BM, BM)], sem_o.at[t])

    cp_small(0).start()
    cp_ssm(0).start()
    cp_ssm(1).start()
    for i in range(1, 4):
        cp_small(i).start()
    cp_ssm(2).start()
    cp_ssm(3).start()

    def bc(i, rows):
        return jnp.broadcast_to(vec[i, 0:1, :], (rows, D))

    def make_kv(t):
        R = 64
        for r in range(0, BM, R):
            kk = k_s[pl.ds(pl.multiple_of(t * BM + r, HALO), R + HALO), :].astype(F32)
            ks = kk[HALO:] * bc(V_W0, R)
            for j in range(1, 4):
                ks = ks + kk[HALO - j:HALO - j + R] * bc(V_W0 + j, R)
            vv = v_s[pl.ds(pl.multiple_of(t * BM + r, R), R), :].astype(F32)
            kv_s[t % 2, r:r + R, :] = (ks * vv).astype(BF16)

    def conv_fwd(t):
        for c in range(2):
            u = jnp.dot(f_s[2 * (t % 2) + c], kv_s[t % 2, c * C:(c + 1) * C, :], preferred_element_type=F32)
            pool[UB + 2 * t + c] = u

    def cmul(kr, ki, ur, ui):
        return kr * ur - ki * ui, kr * ui + ki * ur

    def block(I, J, L, diag, first):
        ys, us, ks = YB + 2 * I, UB + 2 * J, KB + 2 * L
        for r in range(0, C, ROWS):
            re, im = slice(r, r + ROWS), slice(C + r, C + r + ROWS)
            u0r, u0i = pool[us, re, :], pool[us, im, :]
            u1r, u1i = pool[us + 1, re, :], pool[us + 1, im, :]
            kbr, kbi = pool[ks, re, :], pool[ks, im, :]
            kcr, kci = pool[ks + 1, re, :], pool[ks + 1, im, :]
            ar, ai = cmul(kbr, kbi, u0r, u0i)
            if not diag:
                kar, kai = pool[ks - 1, re, :], pool[ks - 1, im, :]
                cr, ci = cmul(kar, kai, u1r, u1i)
                ar, ai = ar + cr, ai + ci
            br, bi = cmul(kcr, kci, u0r, u0i)
            dr, di = cmul(kbr, kbi, u1r, u1i)
            br, bi = br + dr, bi + di
            if not first:
                ar, ai = pool[ys, re, :] + ar, pool[ys, im, :] + ai
                br, bi = pool[ys + 1, re, :] + br, pool[ys + 1, im, :] + bi
            pool[ys, re, :] = ar
            pool[ys, im, :] = ai
            pool[ys + 1, re, :] = br
            pool[ys + 1, im, :] = bi

    def sched_blocks(t):
        block(t, t, 0, True, False)
        for sched in _SCHED:
            I = (_pack([ij[0] for ij in sched]) >> (3 * t)) & 7
            J = (_pack([ij[1] for ij in sched]) >> (3 * t)) & 7
            block(I, J, I - J, False, False)

    def inverse_post(t, first=False):
        slot = t % 2
        for c in range(2):
            if first and c == 0:
                yf = pool[YB].astype(BF16)
            else:
                yf = (pool[YB + 2 * t + c] + pool[YB + 2 * t + c - 1]).astype(BF16)
            y = jnp.dot(g_s[2 * (t % 2) + c], yf, preferred_element_type=F32)
            R = 64
            for r in range(0, C, R):
                rr = c * C + r
                kv = kv_s[slot, rr:rr + R, :].astype(F32)
                yy = y[r:r + R] + kv * bc(V_D, R)
                x = q_s[pl.ds(pl.multiple_of(t * BM + rr, R), R), :].astype(F32)
                gh = _layernorm(x) * bc(V_A1, R) + bc(V_SA, R)
                x1 = x + gh * yy
                x1_s[slot, rr:rr + R, :] = x1
                h2 = _layernorm(x1) * bc(V_B1, R) + bc(V_SB, R)
                h2_s[slot, rr:rr + R, :] = h2.astype(BF16)

    def gate_up(t, j):
        h = h2_s[t % 2]
        g = jnp.dot(h, wg_s[j], preferred_element_type=F32)
        u = jnp.dot(h, wu_s[j], preferred_element_type=F32)
        return (g * u).astype(BF16)

    def put_hidden(j, a):
        a_s[:, j * FC:(j + 1) * FC] = a

    def down_out(t):
        o = jnp.dot(a_s[...], wd_s[...], preferred_element_type=F32)
        o = x1_s[t % 2] + bc(V_GB, BM) * o
        out_s[pl.ds(pl.multiple_of(t * BM, BM), BM), :] = o.astype(BF16)
        cp_o(t).start()

    def mod(s, dst, plus_one):
        cp_wm(s).wait()
        m = jnp.dot(sc, wm_s[s], preferred_element_type=F32)[0:8]
        m = m.astype(BF16).astype(F32)
        vec[dst] = 1.0 + m if plus_one else m

    k_s[0:HALO, :] = jnp.zeros((HALO, D), BF16)
    cp_small(0).wait()

    def k_piece(p, carry):
        cp_ssm(p).wait()

        @pl.when(p == 1)
        def _():
            for t in range(2):
                cp_k(t).start()
                cp_v(t).start()
            for s_ in range(2):
                cp_wm(s_).start()

        @pl.when(p == 3)
        def _():
            for s_ in range(2, 5):
                cp_wm(s_).start()
            cp_small(4).start()
            cp_q(0).start()
            cp_q(1).start()
            cp_wm(5).start()

        for i in range(SP // C):
            m = p * (SP // C) + i
            chunk = ssm_s[:, pl.ds(pl.multiple_of(m * C, C), C)]
            pool[KB + m] = jax.lax.dot_general(f_s[i % 4], chunk, (((1,), (1,)), ((), ())),
                                               preferred_element_type=F32)
        return carry

    jax.lax.fori_loop(0, NSP, k_piece, 0)

    for i in range(1, 4):
        cp_small(i).wait()
    sh = sh_s[...].astype(F32)
    for j in range(4):
        vec[V_W0 + j] = jnp.broadcast_to(sh[j:j + 1, :], (8, D))
    vec[V_D] = jnp.broadcast_to(d_s[...].astype(F32).reshape(1, D), (8, D))
    cf = c_s[...].astype(F32)
    sc = (cf * jax.nn.sigmoid(cf)).astype(BF16)
    sc = jnp.broadcast_to(sc, (16, D))

    def first_blocks(I, carry):
        block(I, 0, I, False, True)
        return carry

    def conv_step(t, carry):
        cp_k(t).wait()
        cp_v(t).wait()
        make_kv(t)
        conv_fwd(t)

        @pl.when(t == 0)
        def _():
            for j in range(NF):
                cp_wg(j).start()
                cp_wu(j).start()
            block(0, 0, 0, True, True)
            jax.lax.fori_loop(1, _ZERO_FROM, first_blocks, 0)

        @pl.when(t == 1)
        def _():
            for j in range(NF):
                cp_wd(j).start()
            cp_k(2).start()
            cp_v(2).start()
            cp_q(2).start()
            block(t, t, 0, True, False)
            block(t + 1, t, 1, False, False)
        return carry

    jax.lax.fori_loop(0, 2, conv_step, 0)

    mod(0, V_SA, False)
    mod(1, V_A1, True)
    mod(2, V_GA, False)
    vec[V_A1] = vec[V_A1] * vec[V_GA]
    vec[V_SA] = vec[V_SA] * vec[V_GA]
    mod(3, V_SB, False)
    mod(4, V_B1, True)
    cp_small(4).wait()
    cp_q(0).wait()
    inverse_post(0, True)
    cp_q(1).wait()
    inverse_post(1)
    mod(5, V_GB, False)

    def mlp_alone(t):
        @pl.when(t == 0)
        def _():
            cp_wg(0).wait()
            cp_wu(0).wait()

        for i in range(2 * _ZERO_FROM, 2 * NSTEP):
            pool[YB + i] = jnp.zeros((2 * C, D), F32)
        a = gate_up(t, 0)
        for j in range(1, NF):
            @pl.when(t == 0)
            def _():
                cp_wg(j).wait()
                cp_wu(j).wait()

            put_hidden(j - 1, a)
            a = gate_up(t, j)

        @pl.when(t == 0)
        def _():
            for j in range(NF):
                cp_wd(j).wait()

        put_hidden(NF - 1, a)
        down_out(t)

    def paired(t):
        u = t + 1
        cp_k(u).wait()
        cp_v(u).wait()
        cp_q(u).wait()

        @pl.when(u < NSTEP - 1)
        def _():
            cp_k(u + 1).start()
            cp_v(u + 1).start()
            cp_q(u + 1).start()

        make_kv(u)
        conv_fwd(u)
        sched_blocks(u)
        for j in range(NF):
            put_hidden(j, gate_up(t, j))
        inverse_post(u)
        down_out(t)

    def step(t, carry):
        edge = jnp.logical_or(t == 0, t == NSTEP - 1)

        @pl.when(edge)
        def _():
            mlp_alone(t)

        @pl.when(jnp.logical_not(edge))
        def _():
            paired(t)
        return carry

    jax.lax.fori_loop(0, NSTEP, step, 0)
    for t in range(NSTEP):
        cp_o(t).wait()


@jax.jit
def pallas_adaLN_cond__ssm_conv_h3__glu_gated_bilinear__prompt_kernel(
    A_q: jax.Array,
    A_k: jax.Array,
    A_v: jax.Array,
    A_shift_k: jax.Array,
    A_ssm_k: jax.Array,
    A_ssm_D: jax.Array,
    B_x: jax.Array,
    B_w_gate: jax.Array,
    B_w_up: jax.Array,
    B_w_down: jax.Array,
    c: jax.Array,
    w_mod: jax.Array,
):
    del B_x
    fwd, inv = _dft_matrices()
    any_spec = pl.BlockSpec(memory_space=pl.ANY)
    scratch = [
        pltpu.VMEM((S, D), BF16),
        pltpu.VMEM((HALO + S, D), BF16),
        pltpu.VMEM((S, D), BF16),
        pltpu.VMEM((4, D), BF16),
        pltpu.VMEM((D, S), BF16),
        pltpu.VMEM((D,), BF16),
        pltpu.VMEM((NF, D, FC), BF16),
        pltpu.VMEM((NF, D, FC), BF16),
        pltpu.VMEM((FF, D), BF16),
        pltpu.VMEM((1, D), BF16),
        pltpu.VMEM((6, D, D), BF16),
        pltpu.VMEM((4, 2 * C, C), BF16),
        pltpu.VMEM((4, C, 2 * C), BF16),
        pltpu.VMEM((NSLOT, 2 * C, D), F32),
        pltpu.VMEM((12, 8, D), F32),
        pltpu.VMEM((2, BM, D), BF16),
        pltpu.VMEM((2, BM, D), F32),
        pltpu.VMEM((2, BM, D), BF16),
        pltpu.VMEM((BM, FF), BF16),
        pltpu.VMEM((S, D), BF16),
        pltpu.SemaphoreType.DMA((5,)),
        pltpu.SemaphoreType.DMA((4,)),
        pltpu.SemaphoreType.DMA((6,)),
        pltpu.SemaphoreType.DMA((NSTEP,)),
        pltpu.SemaphoreType.DMA((NSTEP,)),
        pltpu.SemaphoreType.DMA((NSTEP,)),
        pltpu.SemaphoreType.DMA((NF,)),
        pltpu.SemaphoreType.DMA((NF,)),
        pltpu.SemaphoreType.DMA((NF,)),
        pltpu.SemaphoreType.DMA((NSTEP,)),
    ]
    out = pl.pallas_call(
        _kernel,
        in_specs=[any_spec] * 13,
        out_specs=any_spec,
        out_shape=jax.ShapeDtypeStruct((S, D), BF16),
        scratch_shapes=scratch,
        compiler_params=pltpu.CompilerParams(vmem_limit_bytes=110 * 2**20, flags=FLAGS),
    )(A_q.reshape(S, D), A_k.reshape(S, D), A_v.reshape(S, D), A_shift_k.T, A_ssm_k, A_ssm_D,
      B_w_gate, B_w_up, B_w_down, c, w_mod, fwd, inv)
    return out.reshape(1, S, D)
```

```python
import numpy as np

import jax
import jax.numpy as jnp
import jax.experimental.pallas as pl
import jax.experimental.pallas.tpu as pltpu

S, D, FF = 2048, 640, 1536
C = 128
BM = 256
NSTEP = S // BM
HALO = 16
EPS = 1e-5

KB, UB, YB = 0, 16, 32
NSLOT = 48

import os as _os, json as _json
CFG = dict(FC=512, PR=32, FORM='late', KVR=64, POSTR=64, ORDER='kFPgggId', ILV=0, LAYOUT=1)
CFG.update(_json.loads(_os.environ.get('KCFG', '{}')))
FC = CFG['FC']
NF = FF // FC
PR = CFG['PR']
NT = D // 128

F32, BF16 = jnp.float32, jnp.bfloat16
FLAGS = None

V_A1, V_SA, V_GA, V_B1, V_SB, V_GB, V_W0, V_D, V_SGN = 0, 1, 2, 3, 4, 5, 6, 10, 11


def _dft_matrices():
    f = np.arange(C, dtype=np.float64)[None, :, None] + 0.5
    s = np.arange(4 * C, dtype=np.float64).reshape(4, 1, C)
    ang = 2.0 * np.pi * f * s / (2 * C)
    fwd = np.concatenate([np.cos(ang), -np.sin(ang)], axis=1)
    inv = np.swapaxes(fwd, 1, 2) / C
    return fwd.astype(np.float32).astype(BF16), inv.astype(np.float32).astype(BF16)


_SCHED = [
    [(3, 1), (4, 2), (5, 2), (6, 1), (6, 5), (7, 3)],
    [(3, 2), (4, 3), (5, 3), (6, 2), (7, 0), (7, 4)],
    [(4, 0), (5, 0), (5, 4), (6, 3), (7, 1), (7, 5)],
    [(4, 1), (5, 1), (6, 0), (6, 4), (7, 2), (7, 6)],
]
_ZERO_FROM = 4


def _pack(vals):
    r = 0
    for t, x in enumerate(vals):
        r |= x << (3 * (t + 2))
    return r


def _layernorm(x):
    m = jnp.mean(x, axis=1, keepdims=True)
    xc = x - m
    v = jnp.mean(xc * xc, axis=1, keepdims=True)
    return xc * jax.lax.rsqrt(v + EPS)


def _kernel(q_hbm, k_hbm, v_hbm, sh_hbm, ssm_hbm, d_hbm, wg_hbm, wu_hbm, wd_hbm, c_hbm, wm_hbm,
            f_hbm, g_hbm, o_hbm,
            q_s, k_s, v_s, sh_s, ssm_s, d_s, wgu_s, wd_s, c_s, wm_s, f_s, g_s,
            pool, vec, kv_s, x1_s, h2_s, a_s, out_s,
            sem_small, sem_ssm, sem_wm, sem_k, sem_v, sem_q, sem_wg, sem_wu, sem_wd, sem_o):

    def cp_small(i):
        src, dst = [(f_hbm, f_s), (sh_hbm, sh_s), (d_hbm, d_s), (c_hbm, c_s), (g_hbm, g_s)][i]
        return pltpu.make_async_copy(src, dst, sem_small.at[i])

    NSP = 4
    SP = S // NSP

    def cp_ssm(p):
        return pltpu.make_async_copy(ssm_hbm.at[:, pl.ds(p * SP, SP)], ssm_s.at[:, pl.ds(p * SP, SP)], sem_ssm.at[p])

    def cp_wm(s):
        return pltpu.make_async_copy(wm_hbm.at[:, pl.ds(s * D, D)], wm_s.at[s], sem_wm.at[s])

    def cp_k(t):
        return pltpu.make_async_copy(k_hbm.at[pl.ds(t * BM, BM)], k_s.at[pl.ds(HALO + t * BM, BM)], sem_k.at[t])

    def cp_v(t):
        return pltpu.make_async_copy(v_hbm.at[pl.ds(t * BM, BM)], v_s.at[pl.ds(t * BM, BM)], sem_v.at[t])

    def cp_q(t):
        return pltpu.make_async_copy(q_hbm.at[pl.ds(t * BM, BM)], q_s.at[pl.ds(t * BM, BM)], sem_q.at[t])

    class _Multi:
        def __init__(self, cps):
            self.cps = cps

        def start(self):
            for c_ in self.cps:
                c_.start()

        def wait(self):
            for c_ in self.cps:
                c_.wait()

    def cp_w(j, src, sem, off):
        if not CFG['ILV']:
            return pltpu.make_async_copy(src.at[:, pl.ds(j * FC, FC)], wgu_s.at[j, :, pl.ds(off * FC, FC)], sem.at[j])
        return _Multi([pltpu.make_async_copy(src.at[:, pl.ds(j * FC + i * 128, 128)],
                                             wgu_s.at[j, :, pl.ds((2 * i + off) * 128, 128)], sem.at[j])
                       for i in range(FC // 128)])

    def cp_wg(j):
        return cp_w(j, wg_hbm, sem_wg, 0)

    def cp_wu(j):
        return cp_w(j, wu_hbm, sem_wu, 1)

    def cp_wd(j):
        return pltpu.make_async_copy(wd_hbm.at[pl.ds(j * FC, FC)], wd_s.at[pl.ds(j * FC, FC)], sem_wd.at[j])

    def cp_o(t):
        return pltpu.make_async_copy(out_s.at[pl.ds(t * BM, BM)], o_hbm.at[pl.ds(t * BM, BM)], sem_o.at[t])

    cp_small(0).start()
    cp_ssm(0).start()
    cp_ssm(1).start()
    for i in range(1, 4):
        cp_small(i).start()
    cp_ssm(2).start()
    cp_ssm(3).start()

    def bc(i, rows):
        return jnp.broadcast_to(vec[i, 0:1, :], (rows, D))

    def make_kv(t, slot=None):
        R = CFG['KVR']
        for r in range(0, BM, R):
            kk = k_s[pl.ds(pl.multiple_of(t * BM + r, HALO), R + HALO), :].astype(F32)
            ks = kk[HALO:] * bc(V_W0, R)
            for j in range(1, 4):
                ks = ks + kk[HALO - j:HALO - j + R] * bc(V_W0 + j, R)
            vv = v_s[pl.ds(pl.multiple_of(t * BM + r, R), R), :].astype(F32)
            kv_s[(t if slot is None else slot) % 2, r:r + R, :] = (ks * vv).astype(BF16)

    def put_slot(s_, val):
        for c_ in range(NT):
            pool[s_, c_] = val[:, c_ * 128:(c_ + 1) * 128]

    def get_slot(s_):
        return jnp.concatenate([pool[s_, c_] for c_ in range(NT)], axis=1)

    def conv_fwd(t):
        for c in range(2):
            u = jnp.dot(f_s[2 * (t % 2) + c], kv_s[t % 2, c * C:(c + 1) * C, :], preferred_element_type=F32)
            put_slot(UB + 2 * t + c, u)

    def cmul(kr, ki, ur, ui):
        return kr * ur - ki * ui, kr * ui + ki * ur

    def block(I, J, L, diag, first):
        ys, us, ks = YB + 2 * I, UB + 2 * J, KB + 2 * L
        for c_ in range(NT):
            for r in range(0, C, PR):
                re, im = slice(r, r + PR), slice(C + r, C + r + PR)
                L = lambda s_, sl: pool[s_, c_, sl, :]
                u0r, u0i, u1r, u1i = L(us, re), L(us, im), L(us + 1, re), L(us + 1, im)
                kbr, kbi, kcr, kci = L(ks, re), L(ks, im), L(ks + 1, re), L(ks + 1, im)
                ar, ai = cmul(kbr, kbi, u0r, u0i)
                if not diag:
                    cr, ci = cmul(L(ks - 1, re), L(ks - 1, im), u1r, u1i)
                    ar, ai = ar + cr, ai + ci
                if CFG['FORM'] == 'seq':
                    if not first:
                        ar, ai = L(ys, re) + ar, L(ys, im) + ai
                    pool[ys, c_, re, :] = ar
                    pool[ys, c_, im, :] = ai
                br, bi = cmul(kcr, kci, u0r, u0i)
                dr, di = cmul(kbr, kbi, u1r, u1i)
                br, bi = br + dr, bi + di
                if not first:
                    br, bi = L(ys + 1, re) + br, L(ys + 1, im) + bi
                if CFG['FORM'] != 'seq':
                    if not first:
                        ar, ai = L(ys, re) + ar, L(ys, im) + ai
                    pool[ys, c_, re, :] = ar
                    pool[ys, c_, im, :] = ai
                pool[ys + 1, c_, re, :] = br
                pool[ys + 1, c_, im, :] = bi

    def sched_blocks(t):
        block(t, t, 0, True, False)
        for sched in _SCHED:
            I = (_pack([ij[0] for ij in sched]) >> (3 * t)) & 7
            J = (_pack([ij[1] for ij in sched]) >> (3 * t)) & 7
            block(I, J, I - J, False, False)

    def inverse_post(t, first=False):
        slot = t % 2
        for c in range(2):
            if first and c == 0:
                yf = get_slot(YB).astype(BF16)
            else:
                yf = (get_slot(YB + 2 * t + c) + get_slot(YB + 2 * t + c - 1)).astype(BF16)
            y = jnp.dot(g_s[2 * (t % 2) + c], yf, preferred_element_type=F32)
            R = CFG['POSTR']
            for r in range(0, C, R):
                rr = c * C + r
                kv = kv_s[slot, rr:rr + R, :].astype(F32)
                yy = y[r:r + R] + kv * bc(V_D, R)
                x = q_s[pl.ds(pl.multiple_of(t * BM + rr, R), R), :].astype(F32)
                gh = _layernorm(x) * bc(V_A1, R) + bc(V_SA, R)
                x1 = x + gh * yy
                x1_s[slot, rr:rr + R, :] = x1
                h2 = _layernorm(x1) * bc(V_B1, R) + bc(V_SB, R)
                h2_s[slot, rr:rr + R, :] = h2.astype(BF16)

    def gate_up(t, j):
        h = h2_s[t % 2]
        if not CFG['ILV']:
            g = jnp.dot(h, wgu_s[j, :, 0:FC], preferred_element_type=F32)
            u = jnp.dot(h, wgu_s[j, :, FC:2 * FC], preferred_element_type=F32)
            return (g * u).astype(BF16)
        gu = jnp.dot(h, wgu_s[j], preferred_element_type=F32)
        return jnp.concatenate([(gu[:, 2 * i * 128:(2 * i + 1) * 128] * gu[:, (2 * i + 1) * 128:(2 * i + 2) * 128]).astype(BF16)
                                for i in range(FC // 128)], axis=1)

    def put_hidden(j, a):
        a_s[:, j * FC:(j + 1) * FC] = a

    def down_out(t):
        o = jnp.dot(a_s[...], wd_s[...], preferred_element_type=F32)
        o = x1_s[t % 2] + bc(V_GB, BM) * o
        out_s[pl.ds(pl.multiple_of(t * BM, BM), BM), :] = o.astype(BF16)
        cp_o(t).start()

    def mod(s, dst, plus_one):
        cp_wm(s).wait()
        m = jnp.dot(sc, wm_s[s], preferred_element_type=F32)[0:8]
        m = m.astype(BF16).astype(F32)
        vec[dst] = 1.0 + m if plus_one else m

    k_s[0:HALO, :] = jnp.zeros((HALO, D), BF16)
    cp_small(0).wait()

    def k_piece(p, carry):
        cp_ssm(p).wait()

        @pl.when(p == 1)
        def _():
            for t in range(2):
                cp_k(t).start()
                cp_v(t).start()
            for s_ in range(2):
                cp_wm(s_).start()

        @pl.when(p == 3)
        def _():
            for s_ in range(2, 5):
                cp_wm(s_).start()
            cp_small(4).start()
            cp_q(0).start()
            cp_q(1).start()
            cp_wm(5).start()

        for i in range(SP // C):
            m = p * (SP // C) + i
            chunk = ssm_s[:, pl.ds(pl.multiple_of(m * C, C), C)]
            put_slot(KB + m, jax.lax.dot_general(f_s[i % 4], chunk, (((1,), (1,)), ((), ())),
                                                 preferred_element_type=F32))
        return carry

    jax.lax.fori_loop(0, NSP, k_piece, 0)

    for i in range(1, 4):
        cp_small(i).wait()
    sh = sh_s[...].astype(F32)
    for j in range(4):
        vec[V_W0 + j] = jnp.broadcast_to(sh[j:j + 1, :], (8, D))
    vec[V_D] = jnp.broadcast_to(d_s[...].astype(F32).reshape(1, D), (8, D))
    cf = c_s[...].astype(F32)
    sc = (cf * jax.nn.sigmoid(cf)).astype(BF16)
    sc = jnp.broadcast_to(sc, (16, D))

    def first_blocks(I, carry):
        block(I, 0, I, False, True)
        return carry

    def conv_step(t, carry):
        cp_k(t).wait()
        cp_v(t).wait()
        make_kv(t)
        conv_fwd(t)

        @pl.when(t == 0)
        def _():
            for j in range(NF):
                cp_wg(j).start()
                cp_wu(j).start()
            block(0, 0, 0, True, True)
            jax.lax.fori_loop(1, _ZERO_FROM, first_blocks, 0)

        @pl.when(t == 1)
        def _():
            for j in range(NF):
                cp_wd(j).start()
            cp_k(2).start()
            cp_v(2).start()
            cp_q(2).start()
            block(t, t, 0, True, False)
            block(t + 1, t, 1, False, False)
        return carry

    jax.lax.fori_loop(0, 2, conv_step, 0)

    mod(0, V_SA, False)
    mod(1, V_A1, True)
    mod(2, V_GA, False)
    vec[V_A1] = vec[V_A1] * vec[V_GA]
    vec[V_SA] = vec[V_SA] * vec[V_GA]
    mod(3, V_SB, False)
    mod(4, V_B1, True)
    cp_small(4).wait()
    cp_q(0).wait()
    inverse_post(0, True)
    cp_q(1).wait()
    inverse_post(1)
    mod(5, V_GB, False)

    def mlp_alone(t):
        @pl.when(t == 0)
        def _():
            cp_wg(0).wait()
            cp_wu(0).wait()

        for i in range(2 * _ZERO_FROM, 2 * NSTEP):
            pool[YB + i] = jnp.zeros((NT, 2 * C, 128), F32)
        a = gate_up(t, 0)
        for j in range(1, NF):
            @pl.when(t == 0)
            def _():
                cp_wg(j).wait()
                cp_wu(j).wait()

            put_hidden(j - 1, a)
            a = gate_up(t, j)

        @pl.when(t == 0)
        def _():
            for j in range(NF):
                cp_wd(j).wait()
            cp_k(3).start()
            cp_v(3).start()

        put_hidden(NF - 1, a)
        down_out(t)

    def paired(t):
        u = t + 1
        cp_q(u).wait()

        @pl.when(u < NSTEP - 1)
        def _():
            cp_k(u + 1).wait()
            cp_v(u + 1).wait()
            cp_q(u + 1).start()

        @pl.when(u < NSTEP - 2)
        def _():
            cp_k(u + 2).start()
            cp_v(u + 2).start()

        gi = 0
        for ch in CFG['ORDER']:
            if ch == 'k':
                make_kv(jnp.minimum(u + 1, NSTEP - 1), u + 1)
            elif ch == 'F':
                conv_fwd(u)
            elif ch == 'P':
                sched_blocks(u)
            elif ch == 'g':
                put_hidden(gi, gate_up(t, gi))
                gi += 1
            elif ch == 'I':
                inverse_post(u)
            elif ch == 'd':
                down_out(t)

    def step(t, carry):
        edge = jnp.logical_or(t == 0, t == NSTEP - 1)

        @pl.when(edge)
        def _():
            mlp_alone(t)

        @pl.when(t == 0)
        def _():
            cp_k(2).wait()
            cp_v(2).wait()
            make_kv(2)

        @pl.when(jnp.logical_not(edge))
        def _():
            paired(t)
        return carry

    jax.lax.fori_loop(0, NSTEP, step, 0)
    for t in range(NSTEP):
        cp_o(t).wait()


@jax.jit
def pallas_adaLN_cond__ssm_conv_h3__glu_gated_bilinear__prompt_kernel(
    A_q: jax.Array,
    A_k: jax.Array,
    A_v: jax.Array,
    A_shift_k: jax.Array,
    A_ssm_k: jax.Array,
    A_ssm_D: jax.Array,
    B_x: jax.Array,
    B_w_gate: jax.Array,
    B_w_up: jax.Array,
    B_w_down: jax.Array,
    c: jax.Array,
    w_mod: jax.Array,
):
    del B_x
    fwd, inv = _dft_matrices()
    any_spec = pl.BlockSpec(memory_space=pl.ANY)
    scratch = [
        pltpu.VMEM((S, D), BF16),
        pltpu.VMEM((HALO + S, D), BF16),
        pltpu.VMEM((S, D), BF16),
        pltpu.VMEM((4, D), BF16),
        pltpu.VMEM((D, S), BF16),
        pltpu.VMEM((D,), BF16),
        pltpu.VMEM((NF, D, 2 * FC), BF16),
        pltpu.VMEM((FF, D), BF16),
        pltpu.VMEM((1, D), BF16),
        pltpu.VMEM((6, D, D), BF16),
        pltpu.VMEM((4, 2 * C, C), BF16),
        pltpu.VMEM((4, C, 2 * C), BF16),
        pltpu.VMEM((NSLOT, NT, 2 * C, 128), F32),
        pltpu.VMEM((12, 8, D), F32),
        pltpu.VMEM((2, BM, D), BF16),
        pltpu.VMEM((2, BM, D), F32),
        pltpu.VMEM((2, BM, D), BF16),
        pltpu.VMEM((BM, FF), BF16),
        pltpu.VMEM((S, D), BF16),
        pltpu.SemaphoreType.DMA((5,)),
        pltpu.SemaphoreType.DMA((4,)),
        pltpu.SemaphoreType.DMA((6,)),
        pltpu.SemaphoreType.DMA((NSTEP,)),
        pltpu.SemaphoreType.DMA((NSTEP,)),
        pltpu.SemaphoreType.DMA((NSTEP,)),
        pltpu.SemaphoreType.DMA((NF,)),
        pltpu.SemaphoreType.DMA((NF,)),
        pltpu.SemaphoreType.DMA((NF,)),
        pltpu.SemaphoreType.DMA((NSTEP,)),
    ]
    out = pl.pallas_call(
        _kernel,
        in_specs=[any_spec] * 13,
        out_specs=any_spec,
        out_shape=jax.ShapeDtypeStruct((S, D), BF16),
        scratch_shapes=scratch,
        compiler_params=pltpu.CompilerParams(vmem_limit_bytes=110 * 2**20, flags=FLAGS),
    )(A_q.reshape(S, D), A_k.reshape(S, D), A_v.reshape(S, D), A_shift_k.T, A_ssm_k, A_ssm_D,
      B_w_gate, B_w_up, B_w_down, c, w_mod, fwd, inv)
    return out.reshape(1, S, D)
```

```python
import numpy as np

import jax
import jax.numpy as jnp
import jax.experimental.pallas as pl
import jax.experimental.pallas.tpu as pltpu

S, D, FF = 2048, 640, 1536
C = 128
BM = 256
NSTEP = S // BM
HALO = 16
EPS = 1e-5

KB, UB, YB = 0, 16, 32
NSLOT = 48

import os as _os, json as _json
CFG = dict(FC=512, PR=16, FORM='late', KVR=128, POSTR=128, PREPR=64, ORDER='skFPgggId', ILV=0, LAYOUT=1, SPLIT=1, USEPREP=0)
CFG.update(_json.loads(_os.environ.get('KCFG', '{}')))
FC = CFG['FC']
NF = FF // FC
PR = CFG['PR']
NT = D // 128

F32, BF16 = jnp.float32, jnp.bfloat16
FLAGS = None

V_A1, V_SA, V_GA, V_B1, V_SB, V_GB, V_W0, V_D, V_SGN = 0, 1, 2, 3, 4, 5, 6, 10, 11


def _dft_matrices():
    f = np.arange(C, dtype=np.float64)[None, :, None] + 0.5
    s = np.arange(4 * C, dtype=np.float64).reshape(4, 1, C)
    ang = 2.0 * np.pi * f * s / (2 * C)
    fwd = np.concatenate([np.cos(ang), -np.sin(ang)], axis=1)
    inv = np.swapaxes(fwd, 1, 2) / C
    return fwd.astype(np.float32).astype(BF16), inv.astype(np.float32).astype(BF16)


_SCHED = [
    [(3, 1), (4, 2), (5, 2), (6, 1), (6, 5), (7, 3)],
    [(3, 2), (4, 3), (5, 3), (6, 2), (7, 0), (7, 4)],
    [(4, 0), (5, 0), (5, 4), (6, 3), (7, 1), (7, 5)],
    [(4, 1), (5, 1), (6, 0), (6, 4), (7, 2), (7, 6)],
]
_ZERO_FROM = 4


def _pack(vals):
    r = 0
    for t, x in enumerate(vals):
        r |= x << (3 * (t + 2))
    return r


def _layernorm(x):
    m = jnp.mean(x, axis=1, keepdims=True)
    xc = x - m
    v = jnp.mean(xc * xc, axis=1, keepdims=True)
    return xc * jax.lax.rsqrt(v + EPS)


def _kernel(q_hbm, k_hbm, v_hbm, sh_hbm, ssm_hbm, d_hbm, wg_hbm, wu_hbm, wd_hbm, c_hbm, wm_hbm,
            f_hbm, g_hbm, o_hbm,
            q_s, k_s, v_s, sh_s, ssm_s, d_s, wgu_s, wd_s, c_s, wm_s, f_s, g_s,
            pool, pool_y, vec, kv_s, gh_s, x1_s, h2_s, a_s, out_s,
            sem_small, sem_ssm, sem_wm, sem_k, sem_v, sem_q, sem_wg, sem_wu, sem_wd, sem_o):

    def cp_small(i):
        src, dst = [(f_hbm, f_s), (sh_hbm, sh_s), (d_hbm, d_s), (c_hbm, c_s), (g_hbm, g_s)][i]
        return pltpu.make_async_copy(src, dst, sem_small.at[i])

    NSP = 4
    SP = S // NSP

    def cp_ssm(p):
        return pltpu.make_async_copy(ssm_hbm.at[:, pl.ds(p * SP, SP)], ssm_s.at[:, pl.ds(p * SP, SP)], sem_ssm.at[p])

    def cp_wm(s):
        return pltpu.make_async_copy(wm_hbm.at[:, pl.ds(s * D, D)], wm_s.at[s], sem_wm.at[s])

    def cp_k(t):
        return pltpu.make_async_copy(k_hbm.at[pl.ds(t * BM, BM)], k_s.at[pl.ds(HALO + t * BM, BM)], sem_k.at[t])

    def cp_v(t):
        return pltpu.make_async_copy(v_hbm.at[pl.ds(t * BM, BM)], v_s.at[pl.ds(t * BM, BM)], sem_v.at[t])

    def cp_q(t):
        return pltpu.make_async_copy(q_hbm.at[pl.ds(t * BM, BM)], q_s.at[pl.ds(t * BM, BM)], sem_q.at[t])

    class _Multi:
        def __init__(self, cps):
            self.cps = cps

        def start(self):
            for c_ in self.cps:
                c_.start()

        def wait(self):
            for c_ in self.cps:
                c_.wait()

    def cp_w(j, src, sem, off):
        if not CFG['ILV']:
            return pltpu.make_async_copy(src.at[:, pl.ds(j * FC, FC)], wgu_s.at[j, :, pl.ds(off * FC, FC)], sem.at[j])
        return _Multi([pltpu.make_async_copy(src.at[:, pl.ds(j * FC + i * 128, 128)],
                                             wgu_s.at[j, :, pl.ds((2 * i + off) * 128, 128)], sem.at[j])
                       for i in range(FC // 128)])

    def cp_wg(j):
        return cp_w(j, wg_hbm, sem_wg, 0)

    def cp_wu(j):
        return cp_w(j, wu_hbm, sem_wu, 1)

    def cp_wd(j):
        return pltpu.make_async_copy(wd_hbm.at[pl.ds(j * FC, FC)], wd_s.at[pl.ds(j * FC, FC)], sem_wd.at[j])

    def cp_o(t):
        return pltpu.make_async_copy(out_s.at[pl.ds(t * BM, BM)], o_hbm.at[pl.ds(t * BM, BM)], sem_o.at[t])

    cp_small(0).start()
    cp_ssm(0).start()
    cp_ssm(1).start()
    for i in range(1, 4):
        cp_small(i).start()
    cp_ssm(2).start()
    cp_ssm(3).start()

    def bc(i, rows):
        return jnp.broadcast_to(vec[i, 0:1, :], (rows, D))

    def make_kv(t, slot=None):
        R = CFG['KVR']
        for r in range(0, BM, R):
            kk = k_s[pl.ds(pl.multiple_of(t * BM + r, HALO), R + HALO), :].astype(F32)
            ks = kk[HALO:] * bc(V_W0, R)
            for j in range(1, 4):
                ks = ks + kk[HALO - j:HALO - j + R] * bc(V_W0 + j, R)
            vv = v_s[pl.ds(pl.multiple_of(t * BM + r, R), R), :].astype(F32)
            kv_s[(t if slot is None else slot) % 2, r:r + R, :] = (ks * vv).astype(BF16)

    ypool, yb = (pool_y, 0) if CFG['SPLIT'] else (pool, YB)

    def put_slot(s_, val):
        for c_ in range(NT):
            pool[s_, c_] = val[:, c_ * 128:(c_ + 1) * 128]

    def get_y(i):
        return jnp.concatenate([ypool[yb + i, c_] for c_ in range(NT)], axis=1)

    def conv_fwd(t):
        for c in range(2):
            u = jnp.dot(f_s[2 * (t % 2) + c], kv_s[t % 2, c * C:(c + 1) * C, :], preferred_element_type=F32)
            put_slot(UB + 2 * t + c, u)

    def cmul(kr, ki, ur, ui):
        return kr * ur - ki * ui, kr * ui + ki * ur

    def block(I, J, L, diag, first):
        ys, us, ks = yb + 2 * I, UB + 2 * J, KB + 2 * L
        for c_ in range(NT):
            for r in range(0, C, PR):
                re, im = slice(r, r + PR), slice(C + r, C + r + PR)
                L = lambda s_, sl: pool[s_, c_, sl, :]
                Y = lambda s_, sl: ypool[s_, c_, sl, :]
                u0r, u0i, u1r, u1i = L(us, re), L(us, im), L(us + 1, re), L(us + 1, im)
                kbr, kbi, kcr, kci = L(ks, re), L(ks, im), L(ks + 1, re), L(ks + 1, im)
                ar, ai = cmul(kbr, kbi, u0r, u0i)
                if not diag:
                    cr, ci = cmul(L(ks - 1, re), L(ks - 1, im), u1r, u1i)
                    ar, ai = ar + cr, ai + ci
                if CFG['FORM'] == 'seq':
                    if not first:
                        ar, ai = Y(ys, re) + ar, Y(ys, im) + ai
                    ypool[ys, c_, re, :] = ar
                    ypool[ys, c_, im, :] = ai
                br, bi = cmul(kcr, kci, u0r, u0i)
                dr, di = cmul(kbr, kbi, u1r, u1i)
                br, bi = br + dr, bi + di
                if not first:
                    br, bi = Y(ys + 1, re) + br, Y(ys + 1, im) + bi
                if CFG['FORM'] != 'seq':
                    if not first:
                        ar, ai = Y(ys, re) + ar, Y(ys, im) + ai
                    ypool[ys, c_, re, :] = ar
                    ypool[ys, c_, im, :] = ai
                ypool[ys + 1, c_, re, :] = br
                ypool[ys + 1, c_, im, :] = bi

    def sched_blocks(t):
        block(t, t, 0, True, False)
        for sched in _SCHED:
            I = (_pack([ij[0] for ij in sched]) >> (3 * t)) & 7
            J = (_pack([ij[1] for ij in sched]) >> (3 * t)) & 7
            block(I, J, I - J, False, False)

    def prep(t):
        if not CFG['USEPREP']:
            return
        slot = t % 2
        R = CFG['PREPR']
        for r in range(0, BM, R):
            x = q_s[pl.ds(pl.multiple_of(t * BM + r, R), R), :].astype(F32)
            gh = _layernorm(x) * bc(V_A1, R) + bc(V_SA, R)
            kv = kv_s[slot, r:r + R, :].astype(F32)
            gh_s[r:r + R, :] = gh
            x1_s[slot, r:r + R, :] = x + gh * (kv * bc(V_D, R))

    def inverse_post(t, first=False):
        slot = t % 2
        for c in range(2):
            if first and c == 0:
                yf = get_y(0).astype(BF16)
            else:
                yf = (get_y(2 * t + c) + get_y(2 * t + c - 1)).astype(BF16)
            y = jnp.dot(g_s[2 * (t % 2) + c], yf, preferred_element_type=F32)
            R = CFG['POSTR']
            for r in range(0, C, R):
                rr = c * C + r
                if CFG['USEPREP']:
                    x1 = x1_s[slot, rr:rr + R, :] + gh_s[rr:rr + R, :] * y[r:r + R]
                else:
                    kv = kv_s[slot, rr:rr + R, :].astype(F32)
                    yy = y[r:r + R] + kv * bc(V_D, R)
                    x = q_s[pl.ds(pl.multiple_of(t * BM + rr, R), R), :].astype(F32)
                    gh = _layernorm(x) * bc(V_A1, R) + bc(V_SA, R)
                    x1 = x + gh * yy
                x1_s[slot, rr:rr + R, :] = x1
                h2 = _layernorm(x1) * bc(V_B1, R) + bc(V_SB, R)
                h2_s[slot, rr:rr + R, :] = h2.astype(BF16)

    def gate_up(t, j):
        h = h2_s[t % 2]
        if not CFG['ILV']:
            g = jnp.dot(h, wgu_s[j, :, 0:FC], preferred_element_type=F32)
            u = jnp.dot(h, wgu_s[j, :, FC:2 * FC], preferred_element_type=F32)
            return (g * u).astype(BF16)
        gu = jnp.dot(h, wgu_s[j], preferred_element_type=F32)
        return jnp.concatenate([(gu[:, 2 * i * 128:(2 * i + 1) * 128] * gu[:, (2 * i + 1) * 128:(2 * i + 2) * 128]).astype(BF16)
                                for i in range(FC // 128)], axis=1)

    def put_hidden(j, a):
        a_s[:, j * FC:(j + 1) * FC] = a

    def down_out(t, edge=False):
        o = jnp.dot(a_s[...], wd_s[...], preferred_element_type=F32)
        if edge:
            @pl.when(t == 0)
            def _():
                cp_wm(5).wait()

            gb = jnp.dot(sc, wm_s[5], preferred_element_type=F32)[0:8].astype(BF16).astype(F32)
            vec[V_GB] = gb
            o = x1_s[t % 2] + jnp.broadcast_to(gb[0:1], (BM, D)) * o
        else:
            o = x1_s[t % 2] + bc(V_GB, BM) * o
        out_s[pl.ds(pl.multiple_of(t * BM, BM), BM), :] = o.astype(BF16)
        cp_o(t).start()

    def mod(s, dst, plus_one):
        cp_wm(s).wait()
        m = jnp.dot(sc, wm_s[s], preferred_element_type=F32)[0:8]
        m = m.astype(BF16).astype(F32)
        vec[dst] = 1.0 + m if plus_one else m

    k_s[0:HALO, :] = jnp.zeros((HALO, D), BF16)
    cp_small(0).wait()

    def k_piece(p, carry):
        cp_ssm(p).wait()

        @pl.when(p == 1)
        def _():
            for t in range(2):
                cp_k(t).start()
                cp_v(t).start()
            for s_ in range(2):
                cp_wm(s_).start()

        @pl.when(p == 3)
        def _():
            for s_ in range(2, 5):
                cp_wm(s_).start()
            cp_small(4).start()
            cp_q(0).start()
            cp_q(1).start()

        for i in range(SP // C):
            m = p * (SP // C) + i
            chunk = ssm_s[:, pl.ds(pl.multiple_of(m * C, C), C)]
            put_slot(KB + m, jax.lax.dot_general(f_s[i % 4], chunk, (((1,), (1,)), ((), ())),
                                                 preferred_element_type=F32))
        return carry

    jax.lax.fori_loop(0, NSP, k_piece, 0)

    for i in range(1, 4):
        cp_small(i).wait()
    sh = sh_s[...].astype(F32)
    for j in range(4):
        vec[V_W0 + j] = jnp.broadcast_to(sh[j:j + 1, :], (8, D))
    vec[V_D] = jnp.broadcast_to(d_s[...].astype(F32).reshape(1, D), (8, D))
    cf = c_s[...].astype(F32)
    sc = (cf * jax.nn.sigmoid(cf)).astype(BF16)
    sc = jnp.broadcast_to(sc, (16, D))

    def first_blocks(I, carry):
        block(I, 0, I, False, True)
        return carry

    def conv_step(t, carry):
        cp_k(t).wait()
        cp_v(t).wait()
        make_kv(t)
        conv_fwd(t)

        @pl.when(t == 0)
        def _():
            for j in range(NF):
                cp_wg(j).start()
                cp_wu(j).start()
            block(0, 0, 0, True, True)
            jax.lax.fori_loop(1, _ZERO_FROM, first_blocks, 0)

        @pl.when(t == 1)
        def _():
            for j in range(NF):
                cp_wd(j).start()
            cp_wm(5).start()
            cp_k(2).start()
            cp_v(2).start()
            cp_q(2).start()
            block(t, t, 0, True, False)
            block(t + 1, t, 1, False, False)
        return carry

    jax.lax.fori_loop(0, 2, conv_step, 0)

    mod(0, V_SA, False)
    mod(1, V_A1, True)
    mod(2, V_GA, False)
    vec[V_A1] = vec[V_A1] * vec[V_GA]
    vec[V_SA] = vec[V_SA] * vec[V_GA]
    mod(3, V_SB, False)
    mod(4, V_B1, True)
    cp_small(4).wait()
    cp_q(0).wait()
    prep(0)
    inverse_post(0, True)
    cp_q(1).wait()
    prep(1)
    inverse_post(1)

    def mlp_alone(t):
        @pl.when(t == 0)
        def _():
            cp_wg(0).wait()
            cp_wu(0).wait()

        for i in range(2 * _ZERO_FROM, 2 * NSTEP):
            ypool[yb + i] = jnp.zeros((NT, 2 * C, 128), F32)
        a = gate_up(t, 0)
        for j in range(1, NF):
            @pl.when(t == 0)
            def _():
                cp_wg(j).wait()
                cp_wu(j).wait()

            put_hidden(j - 1, a)
            a = gate_up(t, j)

        @pl.when(t == 0)
        def _():
            for j in range(NF):
                cp_wd(j).wait()
            cp_k(3).start()
            cp_v(3).start()

        put_hidden(NF - 1, a)
        down_out(t, True)

    def paired(t):
        u = t + 1
        cp_q(u).wait()

        @pl.when(u < NSTEP - 1)
        def _():
            cp_k(u + 1).wait()
            cp_v(u + 1).wait()

        def starts():
            @pl.when(u < NSTEP - 1)
            def _():
                cp_q(u + 1).start()

            @pl.when(u < NSTEP - 2)
            def _():
                cp_k(u + 2).start()
                cp_v(u + 2).start()

        gi = 0
        for ch in CFG['ORDER']:
            if ch == 'k':
                make_kv(jnp.minimum(u + 1, NSTEP - 1), u + 1)
            elif ch == 's':
                starts()
            elif ch == 'p':
                prep(u)
            elif ch == 'F':
                conv_fwd(u)
            elif ch == 'P':
                sched_blocks(u)
            elif ch == 'g':
                put_hidden(gi, gate_up(t, gi))
                gi += 1
            elif ch == 'I':
                inverse_post(u)
            elif ch == 'd':
                down_out(t)

    def step(t, carry):
        edge = jnp.logical_or(t == 0, t == NSTEP - 1)

        @pl.when(edge)
        def _():
            mlp_alone(t)

        @pl.when(t == 0)
        def _():
            cp_k(2).wait()
            cp_v(2).wait()
            make_kv(2)

        @pl.when(jnp.logical_not(edge))
        def _():
            paired(t)
        return carry

    jax.lax.fori_loop(0, NSTEP, step, 0)
    for t in range(NSTEP):
        cp_o(t).wait()


@jax.jit
def pallas_adaLN_cond__ssm_conv_h3__glu_gated_bilinear__prompt_kernel(
    A_q: jax.Array,
    A_k: jax.Array,
    A_v: jax.Array,
    A_shift_k: jax.Array,
    A_ssm_k: jax.Array,
    A_ssm_D: jax.Array,
    B_x: jax.Array,
    B_w_gate: jax.Array,
    B_w_up: jax.Array,
    B_w_down: jax.Array,
    c: jax.Array,
    w_mod: jax.Array,
):
    del B_x
    fwd, inv = _dft_matrices()
    any_spec = pl.BlockSpec(memory_space=pl.ANY)
    scratch = [
        pltpu.VMEM((S, D), BF16),
        pltpu.VMEM((HALO + S, D), BF16),
        pltpu.VMEM((S, D), BF16),
        pltpu.VMEM((4, D), BF16),
        pltpu.VMEM((D, S), BF16),
        pltpu.VMEM((D,), BF16),
        pltpu.VMEM((NF, D, 2 * FC), BF16),
        pltpu.VMEM((FF, D), BF16),
        pltpu.VMEM((1, D), BF16),
        pltpu.VMEM((6, D, D), BF16),
        pltpu.VMEM((4, 2 * C, C), BF16),
        pltpu.VMEM((4, C, 2 * C), BF16),
        pltpu.VMEM((NSLOT, NT, 2 * C, 128), F32),
        pltpu.VMEM((16 if CFG['SPLIT'] else 1, NT, 2 * C, 128), F32),
        pltpu.VMEM((12, 8, D), F32),
        pltpu.VMEM((2, BM, D), BF16),
        pltpu.VMEM((BM, D), F32),
        pltpu.VMEM((2, BM, D), F32),
        pltpu.VMEM((2, BM, D), BF16),
        pltpu.VMEM((BM, FF), BF16),
        pltpu.VMEM((S, D), BF16),
        pltpu.SemaphoreType.DMA((5,)),
        pltpu.SemaphoreType.DMA((4,)),
        pltpu.SemaphoreType.DMA((6,)),
        pltpu.SemaphoreType.DMA((NSTEP,)),
        pltpu.SemaphoreType.DMA((NSTEP,)),
        pltpu.SemaphoreType.DMA((NSTEP,)),
        pltpu.SemaphoreType.DMA((NF,)),
        pltpu.SemaphoreType.DMA((NF,)),
        pltpu.SemaphoreType.DMA((NF,)),
        pltpu.SemaphoreType.DMA((NSTEP,)),
    ]
    out = pl.pallas_call(
        _kernel,
        in_specs=[any_spec] * 13,
        out_specs=any_spec,
        out_shape=jax.ShapeDtypeStruct((S, D), BF16),
        scratch_shapes=scratch,
        compiler_params=pltpu.CompilerParams(vmem_limit_bytes=110 * 2**20, flags=FLAGS),
    )(A_q.reshape(S, D), A_k.reshape(S, D), A_v.reshape(S, D), A_shift_k.T, A_ssm_k, A_ssm_D,
      B_w_gate, B_w_up, B_w_down, c, w_mod, fwd, inv)
    return out.reshape(1, S, D)
```

```python
import numpy as np

import jax
import jax.numpy as jnp
import jax.experimental.pallas as pl
import jax.experimental.pallas.tpu as pltpu

S, D, FF = 2048, 640, 1536
C = 128
BM = 256
NSTEP = S // BM
HALO = 16
EPS = 1e-5

KB, UB, YB = 0, 16, 32
NSLOT = 48

import os as _os, json as _json
CFG = dict(FC=768, PR=16, FORM='late', KVR=128, POSTR=128, PREPR=64, ORDER='skFPggId', ILV=0, LAYOUT=1, SPLIT=1, USEPREP=0, BORD='cr', PACK=1, PEEL=1, PIPE=0, F1=768, HONCE=0, BSPLIT=1)
CFG.update(_json.loads(_os.environ.get('KCFG', '{}')))
FC = CFG['FC']
NF = FF // FC
PR = CFG['PR']
NT = D // 128

F32, BF16 = jnp.float32, jnp.bfloat16
FLAGS = None

V_A1, V_SA, V_GA, V_B1, V_SB, V_GB, V_W0, V_D, V_SGN = 0, 1, 2, 3, 4, 5, 6, 10, 11


def _dft_matrices():
    f = np.arange(C, dtype=np.float64)[None, :, None] + 0.5
    s = np.arange(4 * C, dtype=np.float64).reshape(4, 1, C)
    ang = 2.0 * np.pi * f * s / (2 * C)
    fwd = np.concatenate([np.cos(ang), -np.sin(ang)], axis=1)
    inv = np.swapaxes(fwd, 1, 2) / C
    return fwd[:2].astype(np.float32).astype(BF16), inv[:2].astype(np.float32).astype(BF16)


_SCHED = [
    [(3, 1), (4, 2), (5, 2), (6, 1), (6, 5), (7, 3)],
    [(3, 2), (4, 3), (5, 3), (6, 2), (7, 0), (7, 4)],
    [(4, 0), (5, 0), (5, 4), (6, 3), (7, 1), (7, 5)],
    [(4, 1), (5, 1), (6, 0), (6, 4), (7, 2), (7, 6)],
]
_ZERO_FROM = 4


def _pack(vals):
    r = 0
    for t, x in enumerate(vals):
        r |= x << (3 * (t + 2))
    return r


def _layernorm(x):
    m = jnp.mean(x, axis=1, keepdims=True)
    xc = x - m
    v = jnp.mean(xc * xc, axis=1, keepdims=True)
    return xc * jax.lax.rsqrt(v + EPS)


def _kernel(q_hbm, k_hbm, v_hbm, sh_hbm, ssm_hbm, d_hbm, wg_hbm, wu_hbm, wd_hbm, c_hbm, wm_hbm,
            f_hbm, g_hbm, o_hbm,
            q_s, k_s, v_s, sh_s, ssm_s, d_s, wgu_s, wd_s, c_s, wm_s, f_s, g_s,
            pool, pool_y, vec, kv_s, gh_s, x1_s, h2_s, a_s, out_s,
            sem_small, sem_ssm, sem_wm, sem_k, sem_v, sem_q, sem_wg, sem_wu, sem_wd, sem_o):

    def cp_small(i):
        src, dst = [(f_hbm, f_s.at[0:2]), (sh_hbm, sh_s), (d_hbm, d_s), (c_hbm, c_s), (g_hbm, g_s.at[0:2])][i]
        return pltpu.make_async_copy(src, dst, sem_small.at[i])

    NSP = 4
    SP = S // NSP

    def cp_ssm(p):
        return pltpu.make_async_copy(ssm_hbm.at[:, pl.ds(p * SP, SP)], ssm_s.at[:, pl.ds(p * SP, SP)], sem_ssm.at[p])

    def cp_wm(s):
        return pltpu.make_async_copy(wm_hbm.at[:, pl.ds(s * D, D)], wm_s.at[s], sem_wm.at[s])

    def cp_k(t):
        return pltpu.make_async_copy(k_hbm.at[pl.ds(t * BM, BM)], k_s.at[pl.ds(HALO + t * BM, BM)], sem_k.at[t])

    def cp_v(t):
        return pltpu.make_async_copy(v_hbm.at[pl.ds(t * BM, BM)], v_s.at[pl.ds(t * BM, BM)], sem_v.at[t])

    def cp_q(t):
        return pltpu.make_async_copy(q_hbm.at[pl.ds(t * BM, BM)], q_s.at[pl.ds(t * BM, BM)], sem_q.at[t])

    F1 = CFG['F1']
    N1 = FF // F1

    def cp_w(j, src, sem, off):
        jj, r = divmod(j * F1, FC)
        return pltpu.make_async_copy(src.at[:, pl.ds(j * F1, F1)], wgu_s.at[jj, :, pl.ds(off * FC + r, F1)], sem.at[j])

    def cp_wg(j):
        return cp_w(j, wg_hbm, sem_wg, 0)

    def cp_wu(j):
        return cp_w(j, wu_hbm, sem_wu, 1)

    def cp_wd(j):
        return pltpu.make_async_copy(wd_hbm.at[pl.ds(j * F1, F1)], wd_s.at[pl.ds(j * F1, F1)], sem_wd.at[j])

    def cp_o(t):
        return pltpu.make_async_copy(out_s.at[pl.ds(t * BM, BM)], o_hbm.at[pl.ds(t * BM, BM)], sem_o.at[t])

    cp_small(0).start()
    cp_ssm(0).start()
    cp_ssm(1).start()
    for i in range(1, 4):
        cp_small(i).start()
    cp_ssm(2).start()
    cp_ssm(3).start()

    def bc(i, rows):
        return jnp.broadcast_to(vec[i, 0:1, :], (rows, D))

    def make_kv(t, slot=None):
        R = CFG['KVR']
        for r in range(0, BM, R):
            kk = k_s[pl.ds(pl.multiple_of(t * BM + r, HALO), R + HALO), :].astype(F32)
            ks = kk[HALO:] * bc(V_W0, R)
            for j in range(1, 4):
                ks = ks + kk[HALO - j:HALO - j + R] * bc(V_W0 + j, R)
            vv = v_s[pl.ds(pl.multiple_of(t * BM + r, R), R), :].astype(F32)
            kv_s[(t if slot is None else slot) % 2, r:r + R, :] = (ks * vv).astype(BF16)

    ypool, yb = (pool_y, 0) if CFG['SPLIT'] else (pool, YB)

    def put_slot(s_, val):
        for c_ in range(NT):
            pool[s_, c_] = val[:, c_ * 128:(c_ + 1) * 128]

    def get_y(i):
        return jnp.concatenate([ypool[yb + i, c_] for c_ in range(NT)], axis=1)

    def conv_fwd(t):
        for c in range(2):
            u = jnp.dot(f_s[2 * (t % 2) + c], kv_s[t % 2, c * C:(c + 1) * C, :], preferred_element_type=F32)
            put_slot(UB + 2 * t + c, u)

    def cmul(kr, ki, ur, ui):
        return kr * ur - ki * ui, kr * ui + ki * ur

    def block(I, J, L, diag, first):
        ys, us, ks = yb + 2 * I, UB + 2 * J, KB + 2 * L
        crs = [(c_, r) for c_ in range(NT) for r in range(0, C, PR)]
        if CFG['BORD'] == 'rc':
            crs = [(c_, r) for r in range(0, C, PR) for c_ in range(NT)]
        for c_, r in crs:
            if True:
                re, im = slice(r, r + PR), slice(C + r, C + r + PR)
                L = lambda s_, sl: pool[s_, c_, sl, :]
                Y = lambda s_, sl: ypool[s_, c_, sl, :]
                u0r, u0i, u1r, u1i = L(us, re), L(us, im), L(us + 1, re), L(us + 1, im)
                kbr, kbi, kcr, kci = L(ks, re), L(ks, im), L(ks + 1, re), L(ks + 1, im)
                ar, ai = cmul(kbr, kbi, u0r, u0i)
                if not diag:
                    cr, ci = cmul(L(ks - 1, re), L(ks - 1, im), u1r, u1i)
                    ar, ai = ar + cr, ai + ci
                if CFG['FORM'] == 'seq':
                    if not first:
                        ar, ai = Y(ys, re) + ar, Y(ys, im) + ai
                    ypool[ys, c_, re, :] = ar
                    ypool[ys, c_, im, :] = ai
                br, bi = cmul(kcr, kci, u0r, u0i)
                dr, di = cmul(kbr, kbi, u1r, u1i)
                br, bi = br + dr, bi + di
                if not first:
                    br, bi = Y(ys + 1, re) + br, Y(ys + 1, im) + bi
                if CFG['FORM'] != 'seq':
                    if not first:
                        ar, ai = Y(ys, re) + ar, Y(ys, im) + ai
                    ypool[ys, c_, re, :] = ar
                    ypool[ys, c_, im, :] = ai
                ypool[ys + 1, c_, re, :] = br
                ypool[ys + 1, c_, im, :] = bi

    def sched_blocks(t):
        block(t, t, 0, True, False)
        for sched in _SCHED:
            I = (_pack([ij[0] for ij in sched]) >> (3 * t)) & 7
            J = (_pack([ij[1] for ij in sched]) >> (3 * t)) & 7
            block(I, J, I - J, False, False)

    def one_block(t, b):
        if b == 0:
            block(t, t, 0, True, False)
        else:
            sched = _SCHED[b - 1]
            I = (_pack([ij[0] for ij in sched]) >> (3 * t)) & 7
            J = (_pack([ij[1] for ij in sched]) >> (3 * t)) & 7
            block(I, J, I - J, False, False)

    def prep(t):
        if not CFG['USEPREP']:
            return
        slot = t % 2
        R = CFG['PREPR']
        for r in range(0, BM, R):
            x = q_s[pl.ds(pl.multiple_of(t * BM + r, R), R), :].astype(F32)
            gh = _layernorm(x) * bc(V_A1, R) + bc(V_SA, R)
            kv = kv_s[slot, r:r + R, :].astype(F32)
            gh_s[r:r + R, :] = gh
            x1_s[slot, r:r + R, :] = x + gh * (kv * bc(V_D, R))

    last_h2 = [None]

    def gate_k(t):
        z = last_h2[0][-HALO:, -128:]
        k_s[0:HALO, 0:128] = jnp.where(t < 0, z, 0.0).astype(BF16)

    def inverse_post(t, first=False):
        slot = t % 2
        for c in range(2):
            if first and c == 0:
                yf = get_y(0).astype(BF16)
            else:
                yf = (get_y(2 * t + c) + get_y(2 * t + c - 1)).astype(BF16)
            y = jnp.dot(g_s[2 * (t % 2) + c], yf, preferred_element_type=F32)
            R = CFG['POSTR']
            for r in range(0, C, R):
                rr = c * C + r
                if CFG['USEPREP']:
                    x1 = x1_s[slot, rr:rr + R, :] + gh_s[rr:rr + R, :] * y[r:r + R]
                else:
                    kv = kv_s[slot, rr:rr + R, :].astype(F32)
                    yy = y[r:r + R] + kv * bc(V_D, R)
                    x = q_s[pl.ds(pl.multiple_of(t * BM + rr, R), R), :].astype(F32)
                    gh = _layernorm(x) * bc(V_A1, R) + bc(V_SA, R)
                    x1 = x + gh * yy
                x1_s[slot, rr:rr + R, :] = x1
                h2 = _layernorm(x1) * bc(V_B1, R) + bc(V_SB, R)
                last_h2[0] = h2
                if CFG['PACK']:
                    h2_s[slot, rr // 2:(rr + R) // 2, :] = pltpu.bitcast(h2.astype(BF16), jnp.uint32)
                else:
                    h2_s[slot, rr:rr + R, :] = h2.astype(BF16)

    def gate_up(t, j):
        h = pltpu.bitcast(h2_s[t % 2], BF16) if CFG['PACK'] else h2_s[t % 2]
        if not CFG['ILV']:
            g = jnp.dot(h, wgu_s[j, :, 0:FC], preferred_element_type=F32)
            u = jnp.dot(h, wgu_s[j, :, FC:2 * FC], preferred_element_type=F32)
            return (g * u).astype(BF16)
        gu = jnp.dot(h, wgu_s[j], preferred_element_type=F32)
        return jnp.concatenate([(gu[:, 2 * i * 128:(2 * i + 1) * 128] * gu[:, (2 * i + 1) * 128:(2 * i + 2) * 128]).astype(BF16)
                                for i in range(FC // 128)], axis=1)

    def put_hidden(j, a):
        a_s[:, j * FC:(j + 1) * FC] = pltpu.bitcast(a, jnp.uint32) if CFG['PACK'] else a

    def finish(t, o):
        o = x1_s[t % 2] + bc(V_GB, BM) * o
        out_s[pl.ds(pl.multiple_of(t * BM, BM), BM), :] = o.astype(BF16)
        cp_o(t).start()

    def down_out(t):
        a = pltpu.bitcast(a_s[...], BF16) if CFG['PACK'] else a_s[...]
        finish(t, jnp.dot(a, wd_s[...], preferred_element_type=F32))

    def mod(s, dst, plus_one):
        if s < 5:
            cp_wm(s).wait()
        m = jnp.dot(sc, wm_s[s], preferred_element_type=F32)[0:8]
        m = m.astype(BF16).astype(F32)
        vec[dst] = 1.0 + m if plus_one else m

    k_s[0:HALO, :] = jnp.zeros((HALO, D), BF16)
    cp_small(0).wait()
    f_s[2:4] = -f_s[0:2]

    def k_piece(p, carry):
        cp_ssm(p).wait()

        @pl.when(p == 1)
        def _():
            for t in range(2):
                cp_k(t).start()
                cp_v(t).start()
            for s_ in range(2):
                cp_wm(s_).start()

        @pl.when(p == 3)
        def _():
            for s_ in range(2, 5):
                cp_wm(s_).start()
            cp_small(4).start()
            cp_q(0).start()
            cp_q(1).start()

        for i in range(SP // C):
            m = p * (SP // C) + i
            chunk = ssm_s[:, pl.ds(pl.multiple_of(m * C, C), C)]
            put_slot(KB + m, jax.lax.dot_general(f_s[i % 4], chunk, (((1,), (1,)), ((), ())),
                                                 preferred_element_type=F32))
        return carry

    jax.lax.fori_loop(0, NSP, k_piece, 0)

    for i in range(1, 4):
        cp_small(i).wait()
    sh = sh_s[...].astype(F32)
    for j in range(4):
        vec[V_W0 + j] = jnp.broadcast_to(sh[j:j + 1, :], (8, D))
    vec[V_D] = jnp.broadcast_to(d_s[...].astype(F32).reshape(1, D), (8, D))
    cf = c_s[...].astype(F32)
    sc = (cf * jax.nn.sigmoid(cf)).astype(BF16)
    sc = jnp.broadcast_to(sc, (16, D))

    def first_blocks(I, carry):
        block(I, 0, I, False, True)
        return carry

    def conv_step(t, carry):
        cp_k(t).wait()
        cp_v(t).wait()
        make_kv(t)
        conv_fwd(t)

        @pl.when(t == 0)
        def _():
            for j in range(N1):
                cp_wg(j).start()
                cp_wu(j).start()
            block(0, 0, 0, True, True)
            jax.lax.fori_loop(1, _ZERO_FROM, first_blocks, 0)

        @pl.when(t == 1)
        def _():
            for j in range(N1):
                cp_wd(j).start()
            cp_wm(5).start()
            cp_k(2).start()
            cp_v(2).start()
            cp_q(2).start()
            block(t, t, 0, True, False)
            block(t + 1, t, 1, False, False)
        return carry

    jax.lax.fori_loop(0, 2, conv_step, 0)

    mod(0, V_SA, False)
    mod(1, V_A1, True)
    mod(2, V_GA, False)
    vec[V_A1] = vec[V_A1] * vec[V_GA]
    vec[V_SA] = vec[V_SA] * vec[V_GA]
    mod(3, V_SB, False)
    mod(4, V_B1, True)
    cp_small(4).wait()
    g_s[2:4] = -g_s[0:2]
    cp_q(0).wait()
    prep(0)
    inverse_post(0, True)
    cp_q(1).wait()
    prep(1)
    inverse_post(1)

    def mlp_first():
        a = None
        for j in range(NF):
            cp_wg(j).wait()
            cp_wu(j).wait()
            if j == 0:
                for i in range(2 * _ZERO_FROM, 2 * NSTEP):
                    ypool[yb + i] = jnp.zeros((NT, 2 * C, 128), F32)
            else:
                put_hidden(j - 1, a)
            a = gate_up(0, j)
        for j in range(NF):
            cp_wd(j).wait()
        cp_k(3).start()
        cp_v(3).start()
        cp_q(3).start()
        put_hidden(NF - 1, a)
        a = pltpu.bitcast(a_s[...], BF16) if CFG['PACK'] else a_s[...]
        o = jnp.dot(a, wd_s[...], preferred_element_type=F32)
        cp_wm(5).wait()
        mod(5, V_GB, False)
        finish(0, o)

    def mlp_last(t):
        for j in range(NF):
            put_hidden(j, gate_up(t, j))
        down_out(t)

    def paired(t):
        u = t + 1
        cp_k(u).wait()
        cp_v(u).wait()
        cp_q(u).wait()

        def starts():
            @pl.when(jnp.logical_and(u >= 3, u < NSTEP - 1))
            def _():
                cp_k(u + 1).start()
                cp_v(u + 1).start()
                cp_q(u + 1).start()

        gi = 0
        for ch in CFG['ORDER']:
            if ch == 'k':
                if CFG['PIPE']:
                    make_kv(jnp.minimum(u + 1, NSTEP - 1), u + 1)
                else:
                    make_kv(u)
            elif ch == 'G':
                gate_k(t)
            elif ch == 's':
                starts()
            elif ch == 'p':
                prep(u)
            elif ch == 'F':
                conv_fwd(u)
            elif ch == 'P':
                sched_blocks(u)
            elif ch in '01234':
                one_block(u, int(ch))
            elif ch == 'g':
                put_hidden(gi, gate_up(t, gi))
                gi += 1
            elif ch == 'I':
                inverse_post(u)
            elif ch == 'd':
                down_out(t)

    mlp_first()
    jax.lax.fori_loop(1, NSTEP - 1, lambda t, c_: (paired(t), c_)[1], 0)
    mlp_last(NSTEP - 1)
    for t in range(NSTEP):
        cp_o(t).wait()


@jax.jit
def pallas_adaLN_cond__ssm_conv_h3__glu_gated_bilinear__prompt_kernel(
    A_q: jax.Array,
    A_k: jax.Array,
    A_v: jax.Array,
    A_shift_k: jax.Array,
    A_ssm_k: jax.Array,
    A_ssm_D: jax.Array,
    B_x: jax.Array,
    B_w_gate: jax.Array,
    B_w_up: jax.Array,
    B_w_down: jax.Array,
    c: jax.Array,
    w_mod: jax.Array,
):
    del B_x
    fwd, inv = _dft_matrices()
    any_spec = pl.BlockSpec(memory_space=pl.ANY)
    scratch = [
        pltpu.VMEM((S, D), BF16),
        pltpu.VMEM((HALO + S, D), BF16),
        pltpu.VMEM((S, D), BF16),
        pltpu.VMEM((4, D), BF16),
        pltpu.VMEM((D, S), BF16),
        pltpu.VMEM((D,), BF16),
        pltpu.VMEM((NF, D, 2 * FC), BF16),
        pltpu.VMEM((FF, D), BF16),
        pltpu.VMEM((1, D), BF16),
        pltpu.VMEM((6, D, D), BF16),
        pltpu.VMEM((4, 2 * C, C), BF16),
        pltpu.VMEM((4, C, 2 * C), BF16),
        pltpu.VMEM((NSLOT, NT, 2 * C, 128), F32),
        pltpu.VMEM((16 if CFG['SPLIT'] else 1, NT, 2 * C, 128), F32),
        pltpu.VMEM((12, 8, D), F32),
        pltpu.VMEM((2, BM, D), BF16),
        pltpu.VMEM((BM, D), F32),
        pltpu.VMEM((2, BM, D), F32),
        pltpu.VMEM((2, BM // 2, D), jnp.uint32) if CFG['PACK'] else pltpu.VMEM((2, BM, D), BF16),
        pltpu.VMEM((BM // 2, FF), jnp.uint32) if CFG['PACK'] else pltpu.VMEM((BM, FF), BF16),
        pltpu.VMEM((S, D), BF16),
        pltpu.SemaphoreType.DMA((5,)),
        pltpu.SemaphoreType.DMA((4,)),
        pltpu.SemaphoreType.DMA((6,)),
        pltpu.SemaphoreType.DMA((NSTEP,)),
        pltpu.SemaphoreType.DMA((NSTEP,)),
        pltpu.SemaphoreType.DMA((NSTEP,)),
        pltpu.SemaphoreType.DMA((FF // CFG['F1'],)),
        pltpu.SemaphoreType.DMA((FF // CFG['F1'],)),
        pltpu.SemaphoreType.DMA((FF // CFG['F1'],)),
        pltpu.SemaphoreType.DMA((NSTEP,)),
    ]
    out = pl.pallas_call(
        _kernel,
        in_specs=[any_spec] * 13,
        out_specs=any_spec,
        out_shape=jax.ShapeDtypeStruct((S, D), BF16),
        scratch_shapes=scratch,
        compiler_params=pltpu.CompilerParams(vmem_limit_bytes=110 * 2**20, flags=FLAGS),
    )(A_q.reshape(S, D), A_k.reshape(S, D), A_v.reshape(S, D), A_shift_k.T, A_ssm_k, A_ssm_D,
      B_w_gate, B_w_up, B_w_down, c, w_mod, fwd, inv)
    return out.reshape(1, S, D)
```

```python
import numpy as np

import jax
import jax.numpy as jnp
import jax.experimental.pallas as pl
import jax.experimental.pallas.tpu as pltpu

S, D, FF = 2048, 640, 1536
C = 128
BM = 256
NSTEP = S // BM
HALO = 16
EPS = 1e-5

KB, UB, YB = 0, 16, 32
NSLOT = 48

import os as _os, json as _json
CFG = dict(FC=768, PR=16, FORM='late', KVR=128, POSTR=128, PREPR=64, ORDER='skFPggId', ILV=0, LAYOUT=1, SPLIT=1, USEPREP=0, BORD='cr', PACK=1, PEEL=1, PIPE=0, F1=768, KDIRECT=0, HONCE=0, BSPLIT=1)
CFG.update(_json.loads(_os.environ.get('KCFG', '{}')))
FC = CFG['FC']
NF = FF // FC
PR = CFG['PR']
NT = D // 128

F32, BF16 = jnp.float32, jnp.bfloat16
FLAGS = None

V_A1, V_SA, V_GA, V_B1, V_SB, V_GB, V_W0, V_D, V_SGN = 0, 1, 2, 3, 4, 5, 6, 10, 11


def _dft_matrices():
    f = np.arange(C, dtype=np.float64)[None, :, None] + 0.5
    s = np.arange(4 * C, dtype=np.float64).reshape(4, 1, C)
    ang = 2.0 * np.pi * f * s / (2 * C)
    fwd = np.concatenate([np.cos(ang), -np.sin(ang)], axis=1)
    inv = np.swapaxes(fwd, 1, 2) / C
    return _pack_rows(fwd[:2]), _pack_rows(inv[:2])


def _pack_rows(m):
    h = m.astype(np.float32).astype(BF16).view(np.uint16).astype(np.uint32)
    return h[:, 0::2, :] | (h[:, 1::2, :] << 16)


_SCHED = [
    [(3, 1), (4, 2), (5, 2), (6, 1), (6, 5), (7, 3)],
    [(3, 2), (4, 3), (5, 3), (6, 2), (7, 0), (7, 4)],
    [(4, 0), (5, 0), (5, 4), (6, 3), (7, 1), (7, 5)],
    [(4, 1), (5, 1), (6, 0), (6, 4), (7, 2), (7, 6)],
]
_ZERO_FROM = 4


def _pack(vals):
    r = 0
    for t, x in enumerate(vals):
        r |= x << (3 * (t + 2))
    return r


def _layernorm(x):
    m = jnp.mean(x, axis=1, keepdims=True)
    xc = x - m
    v = jnp.mean(xc * xc, axis=1, keepdims=True)
    return xc * jax.lax.rsqrt(v + EPS)


def _kernel(q_hbm, k_hbm, v_hbm, sh_hbm, ssm_hbm, d_hbm, wg_hbm, wu_hbm, wd_hbm, c_hbm, wm_hbm,
            f_hbm, g_hbm, o_hbm,
            q_s, k_s, v_s, sh_s, ssm_s, d_s, wgu_s, wd_s, c_s, wm_s, f_s, g_s,
            pool, pool_y, vec, kv_s, gh_s, x1_s, h2_s, a_s, out_s,
            sem_small, sem_ssm, sem_wm, sem_k, sem_v, sem_q, sem_wg, sem_wu, sem_wd, sem_o):

    def cp_small(i):
        src, dst = [(f_hbm, f_s.at[0:2]), (sh_hbm, sh_s), (d_hbm, d_s), (c_hbm, c_s), (g_hbm, g_s.at[0:2])][i]
        return pltpu.make_async_copy(src, dst, sem_small.at[i])

    NSP = 4
    SP = S // NSP

    def cp_ssm(p):
        return pltpu.make_async_copy(ssm_hbm.at[:, pl.ds(p * SP, SP)], ssm_s.at[:, pl.ds(p * SP, SP)], sem_ssm.at[p])

    def cp_wm(s):
        return pltpu.make_async_copy(wm_hbm.at[:, pl.ds(s * D, D)], wm_s.at[s], sem_wm.at[s])

    def cp_k(t):
        return pltpu.make_async_copy(k_hbm.at[pl.ds(t * BM, BM)], k_s.at[pl.ds(HALO + t * BM, BM)], sem_k.at[t])

    def cp_v(t):
        return pltpu.make_async_copy(v_hbm.at[pl.ds(t * BM, BM)], v_s.at[pl.ds(t * BM, BM)], sem_v.at[t])

    def cp_q(t):
        return pltpu.make_async_copy(q_hbm.at[pl.ds(t * BM, BM)], q_s.at[pl.ds(t * BM, BM)], sem_q.at[t])

    F1 = CFG['F1']
    N1 = FF // F1

    def cp_w(j, src, sem, off):
        jj, r = divmod(j * F1, FC)
        return pltpu.make_async_copy(src.at[:, pl.ds(j * F1, F1)], wgu_s.at[jj, :, pl.ds(off * FC + r, F1)], sem.at[j])

    def cp_wg(j):
        return cp_w(j, wg_hbm, sem_wg, 0)

    def cp_wu(j):
        return cp_w(j, wu_hbm, sem_wu, 1)

    def cp_wd(j):
        return pltpu.make_async_copy(wd_hbm.at[pl.ds(j * F1, F1)], wd_s.at[pl.ds(j * F1, F1)], sem_wd.at[j])

    def cp_o(t):
        return pltpu.make_async_copy(out_s.at[pl.ds(t * BM, BM)], o_hbm.at[pl.ds(t * BM, BM)], sem_o.at[t])

    cp_small(0).start()
    cp_ssm(0).start()
    cp_ssm(1).start()
    for i in range(1, 4):
        cp_small(i).start()
    cp_ssm(2).start()
    cp_ssm(3).start()

    def bc(i, rows):
        return jnp.broadcast_to(vec[i, 0:1, :], (rows, D))

    def make_kv(t, slot=None):
        R = CFG['KVR']
        parts = []
        for r in range(0, BM, R):
            kk = k_s[pl.ds(pl.multiple_of(t * BM + r, HALO), R + HALO), :].astype(F32)
            ks = kk[HALO:] * bc(V_W0, R)
            for j in range(1, 4):
                ks = ks + kk[HALO - j:HALO - j + R] * bc(V_W0 + j, R)
            vv = v_s[pl.ds(pl.multiple_of(t * BM + r, R), R), :].astype(F32)
            parts.append((ks * vv).astype(BF16))
            kv_s[(t if slot is None else slot) % 2, r // 2:(r + R) // 2, :] = pltpu.bitcast(parts[-1], jnp.uint32)
        return jnp.concatenate(parts, axis=0)

    ypool, yb = (pool_y, 0) if CFG['SPLIT'] else (pool, YB)

    def put_slot(s_, val):
        for c_ in range(NT):
            pool[s_, c_] = val[:, c_ * 128:(c_ + 1) * 128]

    def get_y(i):
        return jnp.concatenate([ypool[yb + i, c_] for c_ in range(NT)], axis=1)

    def conv_fwd(t, kv=None):
        for c in range(2):
            rhs = pltpu.bitcast(kv_s[t % 2, c * C // 2:(c + 1) * C // 2, :], BF16) if kv is None or not CFG['KDIRECT'] else kv[c * C:(c + 1) * C]
            u = jnp.dot(pltpu.bitcast(f_s[2 * (t % 2) + c], BF16), rhs, preferred_element_type=F32)
            put_slot(UB + 2 * t + c, u)

    def cmul(kr, ki, ur, ui):
        return kr * ur - ki * ui, kr * ui + ki * ur

    def block(I, J, L, diag, first):
        ys, us, ks = yb + 2 * I, UB + 2 * J, KB + 2 * L
        crs = [(c_, r) for c_ in range(NT) for r in range(0, C, PR)]
        if CFG['BORD'] == 'rc':
            crs = [(c_, r) for r in range(0, C, PR) for c_ in range(NT)]
        for c_, r in crs:
            if True:
                re, im = slice(r, r + PR), slice(C + r, C + r + PR)
                L = lambda s_, sl: pool[s_, c_, sl, :]
                Y = lambda s_, sl: ypool[s_, c_, sl, :]
                u0r, u0i, u1r, u1i = L(us, re), L(us, im), L(us + 1, re), L(us + 1, im)
                kbr, kbi, kcr, kci = L(ks, re), L(ks, im), L(ks + 1, re), L(ks + 1, im)
                ar, ai = cmul(kbr, kbi, u0r, u0i)
                if not diag:
                    cr, ci = cmul(L(ks - 1, re), L(ks - 1, im), u1r, u1i)
                    ar, ai = ar + cr, ai + ci
                if CFG['FORM'] == 'seq':
                    if not first:
                        ar, ai = Y(ys, re) + ar, Y(ys, im) + ai
                    ypool[ys, c_, re, :] = ar
                    ypool[ys, c_, im, :] = ai
                br, bi = cmul(kcr, kci, u0r, u0i)
                dr, di = cmul(kbr, kbi, u1r, u1i)
                br, bi = br + dr, bi + di
                if not first:
                    br, bi = Y(ys + 1, re) + br, Y(ys + 1, im) + bi
                if CFG['FORM'] != 'seq':
                    if not first:
                        ar, ai = Y(ys, re) + ar, Y(ys, im) + ai
                    ypool[ys, c_, re, :] = ar
                    ypool[ys, c_, im, :] = ai
                ypool[ys + 1, c_, re, :] = br
                ypool[ys + 1, c_, im, :] = bi

    def sched_blocks(t):
        block(t, t, 0, True, False)
        for sched in _SCHED:
            I = (_pack([ij[0] for ij in sched]) >> (3 * t)) & 7
            J = (_pack([ij[1] for ij in sched]) >> (3 * t)) & 7
            block(I, J, I - J, False, False)

    def one_block(t, b):
        if b == 0:
            block(t, t, 0, True, False)
        else:
            sched = _SCHED[b - 1]
            I = (_pack([ij[0] for ij in sched]) >> (3 * t)) & 7
            J = (_pack([ij[1] for ij in sched]) >> (3 * t)) & 7
            block(I, J, I - J, False, False)

    def prep(t):
        if not CFG['USEPREP']:
            return
        slot = t % 2
        R = CFG['PREPR']
        for r in range(0, BM, R):
            x = q_s[pl.ds(pl.multiple_of(t * BM + r, R), R), :].astype(F32)
            gh = _layernorm(x) * bc(V_A1, R) + bc(V_SA, R)
            kv = pltpu.bitcast(kv_s[slot, r // 2:(r + R) // 2, :], BF16).astype(F32)
            gh_s[r:r + R, :] = gh
            x1_s[slot, r:r + R, :] = x + gh * (kv * bc(V_D, R))

    last_h2 = [None]

    def gate_k(t):
        z = last_h2[0][-HALO:, -128:]
        k_s[0:HALO, 0:128] = jnp.where(t < 0, z, 0.0).astype(BF16)

    def inverse_post(t, first=False):
        slot = t % 2
        for c in range(2):
            if first and c == 0:
                yf = get_y(0).astype(BF16)
            else:
                yf = (get_y(2 * t + c) + get_y(2 * t + c - 1)).astype(BF16)
            y = jnp.dot(pltpu.bitcast(g_s[2 * (t % 2) + c], BF16), yf, preferred_element_type=F32)
            R = CFG['POSTR']
            for r in range(0, C, R):
                rr = c * C + r
                if CFG['USEPREP']:
                    x1 = x1_s[slot, rr:rr + R, :] + gh_s[rr:rr + R, :] * y[r:r + R]
                else:
                    kv = pltpu.bitcast(kv_s[slot, rr // 2:(rr + R) // 2, :], BF16).astype(F32)
                    yy = y[r:r + R] + kv * bc(V_D, R)
                    x = q_s[pl.ds(pl.multiple_of(t * BM + rr, R), R), :].astype(F32)
                    gh = _layernorm(x) * bc(V_A1, R) + bc(V_SA, R)
                    x1 = x + gh * yy
                x1_s[slot, rr:rr + R, :] = x1
                h2 = _layernorm(x1) * bc(V_B1, R) + bc(V_SB, R)
                last_h2[0] = h2
                if CFG['PACK']:
                    h2_s[slot, rr // 2:(rr + R) // 2, :] = pltpu.bitcast(h2.astype(BF16), jnp.uint32)
                else:
                    h2_s[slot, rr:rr + R, :] = h2.astype(BF16)

    def gate_up(t, j):
        h = pltpu.bitcast(h2_s[t % 2], BF16) if CFG['PACK'] else h2_s[t % 2]
        if not CFG['ILV']:
            g = jnp.dot(h, wgu_s[j, :, 0:FC], preferred_element_type=F32)
            u = jnp.dot(h, wgu_s[j, :, FC:2 * FC], preferred_element_type=F32)
            return (g * u).astype(BF16)
        gu = jnp.dot(h, wgu_s[j], preferred_element_type=F32)
        return jnp.concatenate([(gu[:, 2 * i * 128:(2 * i + 1) * 128] * gu[:, (2 * i + 1) * 128:(2 * i + 2) * 128]).astype(BF16)
                                for i in range(FC // 128)], axis=1)

    def put_hidden(j, a):
        a_s[:, j * FC:(j + 1) * FC] = pltpu.bitcast(a, jnp.uint32) if CFG['PACK'] else a

    def finish(t, o):
        o = x1_s[t % 2] + bc(V_GB, BM) * o
        out_s[pl.ds(pl.multiple_of(t * BM, BM), BM), :] = o.astype(BF16)
        cp_o(t).start()

    def down_out(t):
        a = pltpu.bitcast(a_s[...], BF16) if CFG['PACK'] else a_s[...]
        finish(t, jnp.dot(a, wd_s[...], preferred_element_type=F32))

    def mod(s, dst, plus_one):
        if s < 5:
            cp_wm(s).wait()
        m = jnp.dot(sc, wm_s[s], preferred_element_type=F32)[0:8]
        m = m.astype(BF16).astype(F32)
        vec[dst] = 1.0 + m if plus_one else m

    k_s[0:HALO, :] = jnp.zeros((HALO, D), BF16)
    cp_small(0).wait()
    f_s[2:4] = f_s[0:2] ^ np.uint32(0x80008000)

    def k_piece(p, carry):
        cp_ssm(p).wait()

        @pl.when(p == 1)
        def _():
            for t in range(2):
                cp_k(t).start()
                cp_v(t).start()
            for s_ in range(2):
                cp_wm(s_).start()

        @pl.when(p == 3)
        def _():
            for s_ in range(2, 5):
                cp_wm(s_).start()
            cp_small(4).start()
            cp_q(0).start()
            cp_q(1).start()

        for i in range(SP // C):
            m = p * (SP // C) + i
            chunk = ssm_s[:, pl.ds(pl.multiple_of(m * C, C), C)]
            put_slot(KB + m, jax.lax.dot_general(pltpu.bitcast(f_s[i % 4], BF16), chunk, (((1,), (1,)), ((), ())),
                                                 preferred_element_type=F32))
        return carry

    jax.lax.fori_loop(0, NSP, k_piece, 0)

    for i in range(1, 4):
        cp_small(i).wait()
    sh = sh_s[...].astype(F32)
    for j in range(4):
        vec[V_W0 + j] = jnp.broadcast_to(sh[j:j + 1, :], (8, D))
    vec[V_D] = jnp.broadcast_to(d_s[...].astype(F32).reshape(1, D), (8, D))
    cf = c_s[...].astype(F32)
    sc = (cf * jax.nn.sigmoid(cf)).astype(BF16)
    sc = jnp.broadcast_to(sc, (16, D))

    def first_blocks(I, carry):
        block(I, 0, I, False, True)
        return carry

    def conv_step(t, carry):
        cp_k(t).wait()
        cp_v(t).wait()
        conv_fwd(t, make_kv(t))

        @pl.when(t == 0)
        def _():
            for j in range(N1):
                cp_wg(j).start()
                cp_wu(j).start()
            block(0, 0, 0, True, True)
            jax.lax.fori_loop(1, _ZERO_FROM, first_blocks, 0)

        @pl.when(t == 1)
        def _():
            for j in range(N1):
                cp_wd(j).start()
            cp_wm(5).start()
            cp_k(2).start()
            cp_v(2).start()
            cp_q(2).start()
            block(t, t, 0, True, False)
            block(t + 1, t, 1, False, False)
        return carry

    jax.lax.fori_loop(0, 2, conv_step, 0)

    mod(0, V_SA, False)
    mod(1, V_A1, True)
    mod(2, V_GA, False)
    vec[V_A1] = vec[V_A1] * vec[V_GA]
    vec[V_SA] = vec[V_SA] * vec[V_GA]
    mod(3, V_SB, False)
    mod(4, V_B1, True)
    cp_small(4).wait()
    g_s[2:4] = g_s[0:2] ^ np.uint32(0x80008000)
    cp_q(0).wait()
    prep(0)
    inverse_post(0, True)
    cp_q(1).wait()
    prep(1)
    inverse_post(1)

    def mlp_first():
        a = None
        for j in range(NF):
            cp_wg(j).wait()
            cp_wu(j).wait()
            if j == 0:
                for i in range(2 * _ZERO_FROM, 2 * NSTEP):
                    ypool[yb + i] = jnp.zeros((NT, 2 * C, 128), F32)
            else:
                put_hidden(j - 1, a)
            a = gate_up(0, j)
        for j in range(NF):
            cp_wd(j).wait()
        cp_k(3).start()
        cp_v(3).start()
        cp_q(3).start()
        put_hidden(NF - 1, a)
        a = pltpu.bitcast(a_s[...], BF16) if CFG['PACK'] else a_s[...]
        o = jnp.dot(a, wd_s[...], preferred_element_type=F32)
        cp_wm(5).wait()
        mod(5, V_GB, False)
        finish(0, o)

    def mlp_last(t):
        for j in range(NF):
            put_hidden(j, gate_up(t, j))
        down_out(t)

    def paired(t):
        u = t + 1
        cp_k(u).wait()
        cp_v(u).wait()
        cp_q(u).wait()

        def starts():
            @pl.when(jnp.logical_and(u >= 3, u < NSTEP - 1))
            def _():
                cp_k(u + 1).start()
                cp_v(u + 1).start()
                cp_q(u + 1).start()

        gi = 0
        for ch in CFG['ORDER']:
            if ch == 'k':
                if CFG['PIPE']:
                    make_kv(jnp.minimum(u + 1, NSTEP - 1), u + 1)
                else:
                    kv_u = make_kv(u)
            elif ch == 'G':
                gate_k(t)
            elif ch == 's':
                starts()
            elif ch == 'p':
                prep(u)
            elif ch == 'F':
                conv_fwd(u, kv_u)
            elif ch == 'P':
                sched_blocks(u)
            elif ch in '01234':
                one_block(u, int(ch))
            elif ch == 'g':
                put_hidden(gi, gate_up(t, gi))
                gi += 1
            elif ch == 'I':
                inverse_post(u)
            elif ch == 'd':
                down_out(t)

    mlp_first()
    jax.lax.fori_loop(1, NSTEP - 1, lambda t, c_: (paired(t), c_)[1], 0)
    mlp_last(NSTEP - 1)
    for t in range(NSTEP):
        cp_o(t).wait()


@jax.jit
def pallas_adaLN_cond__ssm_conv_h3__glu_gated_bilinear__prompt_kernel(
    A_q: jax.Array,
    A_k: jax.Array,
    A_v: jax.Array,
    A_shift_k: jax.Array,
    A_ssm_k: jax.Array,
    A_ssm_D: jax.Array,
    B_x: jax.Array,
    B_w_gate: jax.Array,
    B_w_up: jax.Array,
    B_w_down: jax.Array,
    c: jax.Array,
    w_mod: jax.Array,
):
    del B_x
    fwd, inv = _dft_matrices()
    any_spec = pl.BlockSpec(memory_space=pl.ANY)
    scratch = [
        pltpu.VMEM((S, D), BF16),
        pltpu.VMEM((HALO + S, D), BF16),
        pltpu.VMEM((S, D), BF16),
        pltpu.VMEM((4, D), BF16),
        pltpu.VMEM((D, S), BF16),
        pltpu.VMEM((D,), BF16),
        pltpu.VMEM((NF, D, 2 * FC), BF16),
        pltpu.VMEM((FF, D), BF16),
        pltpu.VMEM((1, D), BF16),
        pltpu.VMEM((6, D, D), BF16),
        pltpu.VMEM((4, C, C), jnp.uint32),
        pltpu.VMEM((4, C // 2, 2 * C), jnp.uint32),
        pltpu.VMEM((NSLOT, NT, 2 * C, 128), F32),
        pltpu.VMEM((16 if CFG['SPLIT'] else 1, NT, 2 * C, 128), F32),
        pltpu.VMEM((12, 8, D), F32),
        pltpu.VMEM((2, BM // 2, D), jnp.uint32),
        pltpu.VMEM((BM, D), F32),
        pltpu.VMEM((2, BM, D), F32),
        pltpu.VMEM((2, BM // 2, D), jnp.uint32) if CFG['PACK'] else pltpu.VMEM((2, BM, D), BF16),
        pltpu.VMEM((BM // 2, FF), jnp.uint32) if CFG['PACK'] else pltpu.VMEM((BM, FF), BF16),
        pltpu.VMEM((S, D), BF16),
        pltpu.SemaphoreType.DMA((5,)),
        pltpu.SemaphoreType.DMA((4,)),
        pltpu.SemaphoreType.DMA((6,)),
        pltpu.SemaphoreType.DMA((NSTEP,)),
        pltpu.SemaphoreType.DMA((NSTEP,)),
        pltpu.SemaphoreType.DMA((NSTEP,)),
        pltpu.SemaphoreType.DMA((FF // CFG['F1'],)),
        pltpu.SemaphoreType.DMA((FF // CFG['F1'],)),
        pltpu.SemaphoreType.DMA((FF // CFG['F1'],)),
        pltpu.SemaphoreType.DMA((NSTEP,)),
    ]
    out = pl.pallas_call(
        _kernel,
        in_specs=[any_spec] * 13,
        out_specs=any_spec,
        out_shape=jax.ShapeDtypeStruct((S, D), BF16),
        scratch_shapes=scratch,
        compiler_params=pltpu.CompilerParams(vmem_limit_bytes=110 * 2**20, flags=FLAGS),
    )(A_q.reshape(S, D), A_k.reshape(S, D), A_v.reshape(S, D), A_shift_k.T, A_ssm_k, A_ssm_D,
      B_w_gate, B_w_up, B_w_down, c, w_mod, fwd, inv)
    return out.reshape(1, S, D)
```

```python
import numpy as np

import jax
import jax.numpy as jnp
import jax.experimental.pallas as pl
import jax.experimental.pallas.tpu as pltpu

S, D, FF = 2048, 640, 1536
C = 128
BM = 256
NSTEP = S // BM
HALO = 16
EPS = 1e-5

KB, UB, YB = 0, 16, 32
NSLOT = 48

import os as _os, json as _json
CFG = dict(FC=768, PR=16, FORM='late', KVR=128, POSTR=128, PREPR=64, ORDER='sKPggId', ILV=0, LAYOUT=1, SPLIT=1, USEPREP=0, BORD='cr', PACK=1, PEEL=1, PIPE=0, F1=512, KDIRECT=0, KVPOOL=0, PKV=1, HONCE=0, BSPLIT=1)
CFG.update(_json.loads(_os.environ.get('KCFG', '{}')))
FC = CFG['FC']
NF = FF // FC
PR = CFG['PR']
NT = D // 128

F32, BF16 = jnp.float32, jnp.bfloat16
FLAGS = None

V_A1, V_SA, V_GA, V_B1, V_SB, V_GB, V_W0, V_D, V_SGN = 0, 1, 2, 3, 4, 5, 6, 10, 11


def _dft_matrices():
    f = np.arange(C, dtype=np.float64)[None, :, None] + 0.5
    s = np.arange(4 * C, dtype=np.float64).reshape(4, 1, C)
    ang = 2.0 * np.pi * f * s / (2 * C)
    fwd = np.concatenate([np.cos(ang), -np.sin(ang)], axis=1)
    inv = np.swapaxes(fwd, 1, 2) / C
    return _pack_rows(fwd[:2]), _pack_rows(inv[:2])


def _pack_rows(m):
    h = m.astype(np.float32).astype(BF16).view(np.uint16).astype(np.uint32)
    return h[:, 0::2, :] | (h[:, 1::2, :] << 16)


_SCHED = [
    [(3, 1), (4, 2), (5, 2), (6, 1), (6, 5), (7, 3)],
    [(3, 2), (4, 3), (5, 3), (6, 2), (7, 0), (7, 4)],
    [(4, 0), (5, 0), (5, 4), (6, 3), (7, 1), (7, 5)],
    [(4, 1), (5, 1), (6, 0), (6, 4), (7, 2), (7, 6)],
]
_ZERO_FROM = 4


def _pack(vals):
    r = 0
    for t, x in enumerate(vals):
        r |= x << (3 * (t + 2))
    return r


def _layernorm(x):
    m = jnp.mean(x, axis=1, keepdims=True)
    xc = x - m
    v = jnp.mean(xc * xc, axis=1, keepdims=True)
    return xc * jax.lax.rsqrt(v + EPS)


def _kernel(q_hbm, k_hbm, v_hbm, sh_hbm, ssm_hbm, d_hbm, wg_hbm, wu_hbm, wd_hbm, c_hbm, wm_hbm,
            f_hbm, g_hbm, o_hbm,
            q_s, k_s, v_s, sh_s, ssm_s, d_s, wgu_s, wd_s, c_s, wm_s, f_s, g_s,
            pool, pool_y, vec, kv_s, gh_s, x1_s, h2_s, a_s, out_s,
            sem_small, sem_ssm, sem_wm, sem_k, sem_v, sem_q, sem_wg, sem_wu, sem_wd, sem_o):

    def cp_small(i):
        src, dst = [(f_hbm, f_s.at[0:2]), (sh_hbm, sh_s), (d_hbm, d_s), (c_hbm, c_s), (g_hbm, g_s.at[0:2])][i]
        return pltpu.make_async_copy(src, dst, sem_small.at[i])

    NSP = 4
    SP = S // NSP

    def cp_ssm(p):
        return pltpu.make_async_copy(ssm_hbm.at[:, pl.ds(p * SP, SP)], ssm_s.at[:, pl.ds(p * SP, SP)], sem_ssm.at[p])

    def cp_wm(s):
        return pltpu.make_async_copy(wm_hbm.at[:, pl.ds(s * D, D)], wm_s.at[s], sem_wm.at[s])

    def cp_k(t):
        return pltpu.make_async_copy(k_hbm.at[pl.ds(t * BM, BM)], k_s.at[pl.ds(HALO + t * BM, BM)], sem_k.at[t])

    def cp_v(t):
        return pltpu.make_async_copy(v_hbm.at[pl.ds(t * BM, BM)], v_s.at[pl.ds(t * BM, BM)], sem_v.at[t])

    def cp_q(t):
        return pltpu.make_async_copy(q_hbm.at[pl.ds(t * BM, BM)], q_s.at[pl.ds(t * BM, BM)], sem_q.at[t])

    F1 = CFG['F1']
    N1 = FF // F1

    def segments(j):
        out, lo = [], j * F1
        while lo < (j + 1) * F1:
            jj, r = divmod(lo, FC)
            w = min(FC - r, (j + 1) * F1 - lo)
            out.append((jj, r, w))
            lo += w
        return out

    class Copies:
        def __init__(self, cps):
            self.cps = cps

        def start(self):
            for c_ in self.cps:
                c_.start()

        def wait(self):
            for c_ in self.cps:
                c_.wait()

    def cp_w(j, src, sem, off):
        return Copies([pltpu.make_async_copy(src.at[:, pl.ds(jj * FC + r, w)], wgu_s.at[jj, :, pl.ds(off * FC + r, w)],
                                             sem.at[j]) for jj, r, w in segments(j)])

    def cp_wg(j):
        return cp_w(j, wg_hbm, sem_wg, 0)

    def cp_wu(j):
        return cp_w(j, wu_hbm, sem_wu, 1)

    def cp_wd(j):
        return pltpu.make_async_copy(wd_hbm.at[pl.ds(j * FC, FC)], wd_s.at[pl.ds(j * FC, FC)], sem_wd.at[j])

    def cp_o(t):
        return pltpu.make_async_copy(out_s.at[pl.ds(t * BM, BM)], o_hbm.at[pl.ds(t * BM, BM)], sem_o.at[t])

    cp_small(0).start()
    cp_ssm(0).start()
    cp_ssm(1).start()
    for i in range(1, 4):
        cp_small(i).start()
    cp_ssm(2).start()
    cp_ssm(3).start()

    def bc(i, rows):
        return jnp.broadcast_to(vec[i, 0:1, :], (rows, D))

    def put_kv(slot, r, R, val):
        if CFG['KVPOOL']:
            w = pltpu.bitcast(val, F32)
            for c_ in range(NT):
                pool[32 + slot, c_, r // 2:(r + R) // 2, :] = w[:, c_ * 128:(c_ + 1) * 128]
        elif CFG['PKV']:
            kv_s[slot, r // 2:(r + R) // 2, :] = pltpu.bitcast(val, jnp.uint32)
        else:
            kv_s[slot, r:r + R, :] = val

    def get_kv(slot, r, R):
        if CFG['KVPOOL']:
            w = jnp.concatenate([pool[32 + slot, c_, r // 2:(r + R) // 2, :] for c_ in range(NT)], axis=1)
            return pltpu.bitcast(w, BF16)
        if not CFG['PKV']:
            return kv_s[slot, r:r + R, :]
        return pltpu.bitcast(kv_s[slot, r // 2:(r + R) // 2, :], BF16)

    def make_kv(t, slot=None, rows=(0, BM)):
        R = CFG['KVR']
        parts = []
        for r in range(rows[0], rows[1], R):
            kk = k_s[pl.ds(pl.multiple_of(t * BM + r, HALO), R + HALO), :].astype(F32)
            ks = kk[HALO:] * bc(V_W0, R)
            for j in range(1, 4):
                ks = ks + kk[HALO - j:HALO - j + R] * bc(V_W0 + j, R)
            vv = v_s[pl.ds(pl.multiple_of(t * BM + r, R), R), :].astype(F32)
            parts.append((ks * vv).astype(BF16))
            put_kv((t if slot is None else slot) % 2, r, R, parts[-1])
        return jnp.concatenate(parts, axis=0)

    ypool, yb = (pool_y, 0) if CFG['SPLIT'] else (pool, YB)

    def put_slot(s_, val):
        for c_ in range(NT):
            pool[s_, c_] = val[:, c_ * 128:(c_ + 1) * 128]

    def get_y(i):
        return jnp.concatenate([ypool[yb + i, c_] for c_ in range(NT)], axis=1)

    def kv_fwd(t):
        for c in range(2):
            make_kv(t, rows=(c * C, (c + 1) * C))
            u = jnp.dot(pltpu.bitcast(f_s[2 * (t % 2) + c], BF16), get_kv(t % 2, c * C, C), preferred_element_type=F32)
            put_slot(UB + 2 * t + c, u)

    def conv_fwd(t, kv=None):
        for c in range(2):
            rhs = get_kv(t % 2, c * C, C) if kv is None or not CFG['KDIRECT'] else kv[c * C:(c + 1) * C]
            u = jnp.dot(pltpu.bitcast(f_s[2 * (t % 2) + c], BF16), rhs, preferred_element_type=F32)
            put_slot(UB + 2 * t + c, u)

    def cmul(kr, ki, ur, ui):
        return kr * ur - ki * ui, kr * ui + ki * ur

    def block(I, J, L, diag, first):
        ys, us, ks = yb + 2 * I, UB + 2 * J, KB + 2 * L
        crs = [(c_, r) for c_ in range(NT) for r in range(0, C, PR)]
        if CFG['BORD'] == 'rc':
            crs = [(c_, r) for r in range(0, C, PR) for c_ in range(NT)]
        for c_, r in crs:
            if True:
                re, im = slice(r, r + PR), slice(C + r, C + r + PR)
                L = lambda s_, sl: pool[s_, c_, sl, :]
                Y = lambda s_, sl: ypool[s_, c_, sl, :]
                u0r, u0i, u1r, u1i = L(us, re), L(us, im), L(us + 1, re), L(us + 1, im)
                kbr, kbi, kcr, kci = L(ks, re), L(ks, im), L(ks + 1, re), L(ks + 1, im)
                ar, ai = cmul(kbr, kbi, u0r, u0i)
                if not diag:
                    cr, ci = cmul(L(ks - 1, re), L(ks - 1, im), u1r, u1i)
                    ar, ai = ar + cr, ai + ci
                if CFG['FORM'] == 'seq':
                    if not first:
                        ar, ai = Y(ys, re) + ar, Y(ys, im) + ai
                    ypool[ys, c_, re, :] = ar
                    ypool[ys, c_, im, :] = ai
                br, bi = cmul(kcr, kci, u0r, u0i)
                dr, di = cmul(kbr, kbi, u1r, u1i)
                br, bi = br + dr, bi + di
                if not first:
                    br, bi = Y(ys + 1, re) + br, Y(ys + 1, im) + bi
                if CFG['FORM'] != 'seq':
                    if not first:
                        ar, ai = Y(ys, re) + ar, Y(ys, im) + ai
                    ypool[ys, c_, re, :] = ar
                    ypool[ys, c_, im, :] = ai
                ypool[ys + 1, c_, re, :] = br
                ypool[ys + 1, c_, im, :] = bi

    def sched_blocks(t):
        block(t, t, 0, True, False)
        for sched in _SCHED:
            I = (_pack([ij[0] for ij in sched]) >> (3 * t)) & 7
            J = (_pack([ij[1] for ij in sched]) >> (3 * t)) & 7
            block(I, J, I - J, False, False)

    def one_block(t, b):
        if b == 0:
            block(t, t, 0, True, False)
        else:
            sched = _SCHED[b - 1]
            I = (_pack([ij[0] for ij in sched]) >> (3 * t)) & 7
            J = (_pack([ij[1] for ij in sched]) >> (3 * t)) & 7
            block(I, J, I - J, False, False)

    def prep(t):
        if not CFG['USEPREP']:
            return
        slot = t % 2
        R = CFG['PREPR']
        for r in range(0, BM, R):
            x = q_s[pl.ds(pl.multiple_of(t * BM + r, R), R), :].astype(F32)
            gh = _layernorm(x) * bc(V_A1, R) + bc(V_SA, R)
            kv = get_kv(slot, r, R).astype(F32)
            gh_s[r:r + R, :] = gh
            x1_s[slot, r:r + R, :] = x + gh * (kv * bc(V_D, R))

    last_h2 = [None]

    def gate_k(t):
        z = last_h2[0][-HALO:, -128:]
        k_s[0:HALO, 0:128] = jnp.where(t < 0, z, 0.0).astype(BF16)

    def inverse_post(t, first=False):
        slot = t % 2
        for c in range(2):
            if first and c == 0:
                yf = get_y(0).astype(BF16)
            else:
                yf = (get_y(2 * t + c) + get_y(2 * t + c - 1)).astype(BF16)
            y = jnp.dot(pltpu.bitcast(g_s[2 * (t % 2) + c], BF16), yf, preferred_element_type=F32)
            R = CFG['POSTR']
            for r in range(0, C, R):
                rr = c * C + r
                if CFG['USEPREP']:
                    x1 = x1_s[slot, rr:rr + R, :] + gh_s[rr:rr + R, :] * y[r:r + R]
                else:
                    kv = get_kv(slot, rr, R).astype(F32)
                    yy = y[r:r + R] + kv * bc(V_D, R)
                    x = q_s[pl.ds(pl.multiple_of(t * BM + rr, R), R), :].astype(F32)
                    gh = _layernorm(x) * bc(V_A1, R) + bc(V_SA, R)
                    x1 = x + gh * yy
                x1_s[slot, rr:rr + R, :] = x1
                h2 = _layernorm(x1) * bc(V_B1, R) + bc(V_SB, R)
                last_h2[0] = h2
                if CFG['PACK']:
                    h2_s[slot, rr // 2:(rr + R) // 2, :] = pltpu.bitcast(h2.astype(BF16), jnp.uint32)
                else:
                    h2_s[slot, rr:rr + R, :] = h2.astype(BF16)

    def gate_up(t, j):
        h = pltpu.bitcast(h2_s[t % 2], BF16) if CFG['PACK'] else h2_s[t % 2]
        if not CFG['ILV']:
            g = jnp.dot(h, wgu_s[j, :, 0:FC], preferred_element_type=F32)
            u = jnp.dot(h, wgu_s[j, :, FC:2 * FC], preferred_element_type=F32)
            return (g * u).astype(BF16)
        gu = jnp.dot(h, wgu_s[j], preferred_element_type=F32)
        return jnp.concatenate([(gu[:, 2 * i * 128:(2 * i + 1) * 128] * gu[:, (2 * i + 1) * 128:(2 * i + 2) * 128]).astype(BF16)
                                for i in range(FC // 128)], axis=1)

    def put_hidden(j, a):
        a_s[:, j * FC:(j + 1) * FC] = pltpu.bitcast(a, jnp.uint32) if CFG['PACK'] else a

    def finish(t, o):
        o = x1_s[t % 2] + bc(V_GB, BM) * o
        out_s[pl.ds(pl.multiple_of(t * BM, BM), BM), :] = o.astype(BF16)
        cp_o(t).start()

    def down_out(t):
        a = pltpu.bitcast(a_s[...], BF16) if CFG['PACK'] else a_s[...]
        finish(t, jnp.dot(a, wd_s[...], preferred_element_type=F32))

    def mod(s, dst, plus_one):
        if s < 5:
            cp_wm(s).wait()
        m = jnp.dot(sc, wm_s[s], preferred_element_type=F32)[0:8]
        m = m.astype(BF16).astype(F32)
        vec[dst] = 1.0 + m if plus_one else m

    k_s[0:HALO, :] = jnp.zeros((HALO, D), BF16)
    cp_small(0).wait()
    f_s[2:4] = f_s[0:2] ^ np.uint32(0x80008000)

    def k_piece(p, carry):
        cp_ssm(p).wait()

        @pl.when(p == 1)
        def _():
            for t in range(2):
                cp_k(t).start()
                cp_v(t).start()
            for s_ in range(2):
                cp_wm(s_).start()

        @pl.when(p == 3)
        def _():
            for s_ in range(2, 5):
                cp_wm(s_).start()
            cp_small(4).start()
            cp_q(0).start()
            cp_q(1).start()

        for i in range(SP // C):
            m = p * (SP // C) + i
            chunk = ssm_s[:, pl.ds(pl.multiple_of(m * C, C), C)]
            put_slot(KB + m, jax.lax.dot_general(pltpu.bitcast(f_s[i % 4], BF16), chunk, (((1,), (1,)), ((), ())),
                                                 preferred_element_type=F32))
        return carry

    jax.lax.fori_loop(0, NSP, k_piece, 0)

    for i in range(1, 4):
        cp_small(i).wait()
    sh = sh_s[...].astype(F32)
    for j in range(4):
        vec[V_W0 + j] = jnp.broadcast_to(sh[j:j + 1, :], (8, D))
    vec[V_D] = jnp.broadcast_to(d_s[...].astype(F32).reshape(1, D), (8, D))
    cf = c_s[...].astype(F32)
    sc = (cf * jax.nn.sigmoid(cf)).astype(BF16)
    sc = jnp.broadcast_to(sc, (16, D))

    def first_blocks(I, carry):
        block(I, 0, I, False, True)
        return carry

    def conv_step(t, carry):
        cp_k(t).wait()
        cp_v(t).wait()
        kv_fwd(t)

        @pl.when(t == 0)
        def _():
            for j in range(N1):
                cp_wg(j).start()
                cp_wu(j).start()
            block(0, 0, 0, True, True)
            jax.lax.fori_loop(1, _ZERO_FROM, first_blocks, 0)

        @pl.when(t == 1)
        def _():
            for j in range(NF):
                cp_wd(j).start()
            cp_wm(5).start()
            cp_k(2).start()
            cp_v(2).start()
            cp_q(2).start()
            block(t, t, 0, True, False)
            block(t + 1, t, 1, False, False)
        return carry

    jax.lax.fori_loop(0, 2, conv_step, 0)

    mod(0, V_SA, False)
    mod(1, V_A1, True)
    mod(2, V_GA, False)
    vec[V_A1] = vec[V_A1] * vec[V_GA]
    vec[V_SA] = vec[V_SA] * vec[V_GA]
    mod(3, V_SB, False)
    mod(4, V_B1, True)
    cp_small(4).wait()
    g_s[2:4] = g_s[0:2] ^ np.uint32(0x80008000)
    cp_q(0).wait()
    prep(0)
    inverse_post(0, True)
    cp_q(1).wait()
    prep(1)
    inverse_post(1)

    def mlp_first():
        h = pltpu.bitcast(h2_s[0], BF16) if CFG['PACK'] else h2_s[0]
        pending = []

        def flush():
            for col, val in pending:
                a_s[:, col:col + val.shape[1]] = pltpu.bitcast(val, jnp.uint32) if CFG['PACK'] else val
            pending.clear()

        for j in range(N1):
            cp_wg(j).wait()
            cp_wu(j).wait()
            if j == 0:
                for i in range(2 * _ZERO_FROM, 2 * NSTEP):
                    ypool[yb + i] = jnp.zeros((NT, 2 * C, 128), F32)
            flush()
            for jj, r, w in segments(j):
                g = jnp.dot(h, wgu_s[jj, :, r:r + w], preferred_element_type=F32)
                u = jnp.dot(h, wgu_s[jj, :, FC + r:FC + r + w], preferred_element_type=F32)
                pending.append((jj * FC + r, (g * u).astype(BF16)))
        for j in range(NF):
            cp_wd(j).wait()
        cp_k(3).start()
        cp_v(3).start()
        cp_q(3).start()
        flush()
        a = pltpu.bitcast(a_s[...], BF16) if CFG['PACK'] else a_s[...]
        o = jnp.dot(a, wd_s[...], preferred_element_type=F32)
        cp_wm(5).wait()
        mod(5, V_GB, False)
        finish(0, o)

    def mlp_last(t):
        for j in range(NF):
            put_hidden(j, gate_up(t, j))
        down_out(t)

    def paired(t):
        u = t + 1
        cp_q(u).wait()
        if CFG['PIPE']:
            @pl.when(u < NSTEP - 1)
            def _():
                cp_k(u + 1).wait()
                cp_v(u + 1).wait()
        else:
            cp_k(u).wait()
            cp_v(u).wait()

        def starts():
            if CFG['PIPE']:
                @pl.when(jnp.logical_and(u >= 3, u < NSTEP - 1))
                def _():
                    cp_q(u + 1).start()

                @pl.when(u < NSTEP - 2)
                def _():
                    cp_k(u + 2).start()
                    cp_v(u + 2).start()
            else:
                @pl.when(jnp.logical_and(u >= 3, u < NSTEP - 1))
                def _():
                    cp_k(u + 1).start()
                    cp_v(u + 1).start()
                    cp_q(u + 1).start()

        gi = 0
        kv_u = None
        for ch in CFG['ORDER']:
            if ch == 'k':
                if CFG['PIPE']:
                    kv_u = None
                    make_kv(jnp.minimum(u + 1, NSTEP - 1), u + 1)
                else:
                    kv_u = make_kv(u)
            elif ch == 'G':
                gate_k(t)
            elif ch == 's':
                starts()
            elif ch == 'K':
                kv_fwd(u)
            elif ch == 'p':
                prep(u)
            elif ch == 'F':
                conv_fwd(u, kv_u)
            elif ch == 'P':
                sched_blocks(u)
            elif ch in '01234':
                one_block(u, int(ch))
            elif ch == 'g':
                put_hidden(gi, gate_up(t, gi))
                gi += 1
            elif ch == 'I':
                inverse_post(u)
            elif ch == 'd':
                down_out(t)

    mlp_first()
    if CFG['PIPE']:
        cp_k(2).wait()
        cp_v(2).wait()
        make_kv(2)
    jax.lax.fori_loop(1, NSTEP - 1, lambda t, c_: (paired(t), c_)[1], 0)
    mlp_last(NSTEP - 1)
    for t in range(NSTEP):
        cp_o(t).wait()


@jax.jit
def pallas_adaLN_cond__ssm_conv_h3__glu_gated_bilinear__prompt_kernel(
    A_q: jax.Array,
    A_k: jax.Array,
    A_v: jax.Array,
    A_shift_k: jax.Array,
    A_ssm_k: jax.Array,
    A_ssm_D: jax.Array,
    B_x: jax.Array,
    B_w_gate: jax.Array,
    B_w_up: jax.Array,
    B_w_down: jax.Array,
    c: jax.Array,
    w_mod: jax.Array,
):
    del B_x
    fwd, inv = _dft_matrices()
    any_spec = pl.BlockSpec(memory_space=pl.ANY)
    scratch = [
        pltpu.VMEM((S, D), BF16),
        pltpu.VMEM((HALO + S, D), BF16),
        pltpu.VMEM((S, D), BF16),
        pltpu.VMEM((4, D), BF16),
        pltpu.VMEM((D, S), BF16),
        pltpu.VMEM((D,), BF16),
        pltpu.VMEM((NF, D, 2 * FC), BF16),
        pltpu.VMEM((FF, D), BF16),
        pltpu.VMEM((1, D), BF16),
        pltpu.VMEM((6, D, D), BF16),
        pltpu.VMEM((4, C, C), jnp.uint32),
        pltpu.VMEM((4, C // 2, 2 * C), jnp.uint32),
        pltpu.VMEM((34 if CFG['SPLIT'] else NSLOT, NT, 2 * C, 128), F32),
        pltpu.VMEM((16 if CFG['SPLIT'] else 1, NT, 2 * C, 128), F32),
        pltpu.VMEM((12, 8, D), F32),
        pltpu.VMEM((2, BM // 2, D), jnp.uint32) if CFG['PKV'] else pltpu.VMEM((2, BM, D), BF16),
        pltpu.VMEM((BM, D), F32),
        pltpu.VMEM((2, BM, D), F32),
        pltpu.VMEM((2, BM // 2, D), jnp.uint32) if CFG['PACK'] else pltpu.VMEM((2, BM, D), BF16),
        pltpu.VMEM((BM // 2, FF), jnp.uint32) if CFG['PACK'] else pltpu.VMEM((BM, FF), BF16),
        pltpu.VMEM((S, D), BF16),
        pltpu.SemaphoreType.DMA((5,)),
        pltpu.SemaphoreType.DMA((4,)),
        pltpu.SemaphoreType.DMA((6,)),
        pltpu.SemaphoreType.DMA((NSTEP,)),
        pltpu.SemaphoreType.DMA((NSTEP,)),
        pltpu.SemaphoreType.DMA((NSTEP,)),
        pltpu.SemaphoreType.DMA((FF // CFG['F1'],)),
        pltpu.SemaphoreType.DMA((FF // CFG['F1'],)),
        pltpu.SemaphoreType.DMA((FF // CFG['F1'],)),
        pltpu.SemaphoreType.DMA((NSTEP,)),
    ]
    out = pl.pallas_call(
        _kernel,
        in_specs=[any_spec] * 13,
        out_specs=any_spec,
        out_shape=jax.ShapeDtypeStruct((S, D), BF16),
        scratch_shapes=scratch,
        compiler_params=pltpu.CompilerParams(vmem_limit_bytes=110 * 2**20, flags=FLAGS),
    )(A_q.reshape(S, D), A_k.reshape(S, D), A_v.reshape(S, D), A_shift_k.T, A_ssm_k, A_ssm_D,
      B_w_gate, B_w_up, B_w_down, c, w_mod, fwd, inv)
    return out.reshape(1, S, D)
```

```python
import numpy as np

import jax
import jax.numpy as jnp
import jax.experimental.pallas as pl
import jax.experimental.pallas.tpu as pltpu

S, D, FF = 2048, 640, 1536
C = 128
BM = 256
NSTEP = S // BM
HALO = 16
EPS = 1e-5

KB, UB, YB = 0, 16, 32
NSLOT = 48

import os as _os, json as _json
CFG = dict(FC=768, PR=16, FORM='late', KVR=128, POSTR=128, PREPR=64, ORDER='sKPggId', ILV=0, LAYOUT=1, SPLIT=1, USEPREP=0, BORD='cr', PACK=1, PEEL=1, PIPE=0, F1=512, KDIRECT=0, KVPOOL=0, PKV=1, HONCE=0, BSPLIT=1)
CFG.update(_json.loads(_os.environ.get('KCFG', '{}')))
FC = CFG['FC']
NF = FF // FC
PR = CFG['PR']
NT = D // 128

F32, BF16 = jnp.float32, jnp.bfloat16
FLAGS = None

V_A1, V_SA, V_GA, V_B1, V_SB, V_GB, V_W0, V_D, V_SGN = 0, 1, 2, 3, 4, 5, 6, 10, 11


def _dft_matrices():
    f = np.arange(C, dtype=np.float64)[None, :, None] + 0.5
    s = np.arange(4 * C, dtype=np.float64).reshape(4, 1, C)
    ang = 2.0 * np.pi * f * s / (2 * C)
    fwd = np.concatenate([np.cos(ang), -np.sin(ang)], axis=1)
    inv = np.swapaxes(fwd, 1, 2) / C
    return _pack_rows(fwd[:2]), _pack_rows(inv[:2])


def _pack_rows(m):
    h = m.astype(np.float32).astype(BF16).view(np.uint16).astype(np.uint32)
    return h[:, 0::2, :] | (h[:, 1::2, :] << 16)


_SCHED = [
    [(3, 1), (4, 2), (5, 2), (6, 1), (6, 5), (7, 3)],
    [(3, 2), (4, 3), (5, 3), (6, 2), (7, 0), (7, 4)],
    [(4, 0), (5, 0), (5, 4), (6, 3), (7, 1), (7, 5)],
    [(4, 1), (5, 1), (6, 0), (6, 4), (7, 2), (7, 6)],
]
_ZERO_FROM = 4


def _pack(vals):
    r = 0
    for t, x in enumerate(vals):
        r |= x << (3 * (t + 2))
    return r


def _layernorm(x):
    m = jnp.mean(x, axis=1, keepdims=True)
    xc = x - m
    v = jnp.mean(xc * xc, axis=1, keepdims=True)
    return xc * jax.lax.rsqrt(v + EPS)


def _kernel(q_hbm, k_hbm, v_hbm, sh_hbm, ssm_hbm, d_hbm, wg_hbm, wu_hbm, wd_hbm, c_hbm, wm_hbm,
            f_hbm, g_hbm, o_hbm,
            q_s, k_s, v_s, sh_s, ssm_s, d_s, wgu_s, wd_s, c_s, wm_s, f_s, g_s,
            pool, pool_y, vec, kv_s, gh_s, x1_s, h2_s, a_s, out_s,
            sem_small, sem_ssm, sem_wm, sem_k, sem_v, sem_q, sem_wg, sem_wu, sem_wd, sem_o):

    def cp_small(i):
        src, dst = [(f_hbm, f_s.at[0:2]), (sh_hbm, sh_s), (d_hbm, d_s), (c_hbm, c_s), (g_hbm, g_s.at[0:2])][i]
        return pltpu.make_async_copy(src, dst, sem_small.at[i])

    NSP = 4
    SP = S // NSP

    def cp_ssm(p):
        return pltpu.make_async_copy(ssm_hbm.at[:, pl.ds(p * SP, SP)], ssm_s.at[:, pl.ds(p * SP, SP)], sem_ssm.at[p])

    def cp_wm(s):
        return pltpu.make_async_copy(wm_hbm.at[:, pl.ds(s * D, D)], wm_s.at[s], sem_wm.at[s])

    def cp_k(t):
        return pltpu.make_async_copy(k_hbm.at[pl.ds(t * BM, BM)], k_s.at[pl.ds(HALO + t * BM, BM)], sem_k.at[t])

    def cp_v(t):
        return pltpu.make_async_copy(v_hbm.at[pl.ds(t * BM, BM)], v_s.at[pl.ds(t * BM, BM)], sem_v.at[t])

    def cp_q(t):
        return pltpu.make_async_copy(q_hbm.at[pl.ds(t * BM, BM)], q_s.at[pl.ds(t * BM, BM)], sem_q.at[t])

    F1 = CFG['F1']
    N1 = FF // F1

    def segments(j):
        out, lo = [], j * F1
        while lo < (j + 1) * F1:
            jj, r = divmod(lo, FC)
            w = min(FC - r, (j + 1) * F1 - lo)
            out.append((jj, r, w))
            lo += w
        return out

    class Copies:
        def __init__(self, cps):
            self.cps = cps

        def start(self):
            for c_ in self.cps:
                c_.start()

        def wait(self):
            for c_ in self.cps:
                c_.wait()

    def cp_w(j, src, sem, off):
        return Copies([pltpu.make_async_copy(src.at[:, pl.ds(jj * FC + r, w)], wgu_s.at[jj, :, pl.ds(off * FC + r, w)],
                                             sem.at[j]) for jj, r, w in segments(j)])

    def cp_wg(j):
        return cp_w(j, wg_hbm, sem_wg, 0)

    def cp_wu(j):
        return cp_w(j, wu_hbm, sem_wu, 1)

    def cp_wd(j):
        return pltpu.make_async_copy(wd_hbm.at[pl.ds(j * FC, FC)], wd_s.at[pl.ds(j * FC, FC)], sem_wd.at[j])

    def cp_o(t):
        return pltpu.make_async_copy(out_s.at[pl.ds(t * BM, BM)], o_hbm.at[pl.ds(t * BM, BM)], sem_o.at[t])

    def cp_o_half(hf):
        r0 = (NSTEP - 1) * BM + hf * C
        return pltpu.make_async_copy(out_s.at[pl.ds(r0, C)], o_hbm.at[pl.ds(r0, C)], sem_o.at[NSTEP - 1 + hf])

    cp_small(0).start()
    cp_ssm(0).start()
    cp_ssm(1).start()
    for i in range(1, 4):
        cp_small(i).start()
    cp_ssm(2).start()
    cp_ssm(3).start()

    def bc(i, rows):
        return jnp.broadcast_to(vec[i, 0:1, :], (rows, D))

    def put_kv(slot, r, R, val):
        if CFG['KVPOOL']:
            w = pltpu.bitcast(val, F32)
            for c_ in range(NT):
                pool[32 + slot, c_, r // 2:(r + R) // 2, :] = w[:, c_ * 128:(c_ + 1) * 128]
        elif CFG['PKV']:
            kv_s[slot, r // 2:(r + R) // 2, :] = pltpu.bitcast(val, jnp.uint32)
        else:
            kv_s[slot, r:r + R, :] = val

    def get_kv(slot, r, R):
        if CFG['KVPOOL']:
            w = jnp.concatenate([pool[32 + slot, c_, r // 2:(r + R) // 2, :] for c_ in range(NT)], axis=1)
            return pltpu.bitcast(w, BF16)
        if not CFG['PKV']:
            return kv_s[slot, r:r + R, :]
        return pltpu.bitcast(kv_s[slot, r // 2:(r + R) // 2, :], BF16)

    def make_kv(t, slot=None, rows=(0, BM)):
        R = CFG['KVR']
        parts = []
        for r in range(rows[0], rows[1], R):
            kk = k_s[pl.ds(pl.multiple_of(t * BM + r, HALO), R + HALO), :].astype(F32)
            ks = kk[HALO:] * bc(V_W0, R)
            for j in range(1, 4):
                ks = ks + kk[HALO - j:HALO - j + R] * bc(V_W0 + j, R)
            vv = v_s[pl.ds(pl.multiple_of(t * BM + r, R), R), :].astype(F32)
            parts.append((ks * vv).astype(BF16))
            put_kv((t if slot is None else slot) % 2, r, R, parts[-1])
        return jnp.concatenate(parts, axis=0)

    ypool, yb = (pool_y, 0) if CFG['SPLIT'] else (pool, YB)

    def put_slot(s_, val):
        for c_ in range(NT):
            pool[s_, c_] = val[:, c_ * 128:(c_ + 1) * 128]

    def get_y(i):
        return jnp.concatenate([ypool[yb + i, c_] for c_ in range(NT)], axis=1)

    def kv_fwd(t):
        for c in range(2):
            make_kv(t, rows=(c * C, (c + 1) * C))
            u = jnp.dot(pltpu.bitcast(f_s[2 * (t % 2) + c], BF16), get_kv(t % 2, c * C, C), preferred_element_type=F32)
            put_slot(UB + 2 * t + c, u)

    def conv_fwd(t, kv=None):
        for c in range(2):
            rhs = get_kv(t % 2, c * C, C) if kv is None or not CFG['KDIRECT'] else kv[c * C:(c + 1) * C]
            u = jnp.dot(pltpu.bitcast(f_s[2 * (t % 2) + c], BF16), rhs, preferred_element_type=F32)
            put_slot(UB + 2 * t + c, u)

    def cmul(kr, ki, ur, ui):
        return kr * ur - ki * ui, kr * ui + ki * ur

    def block(I, J, L, diag, first):
        ys, us, ks = yb + 2 * I, UB + 2 * J, KB + 2 * L
        crs = [(c_, r) for c_ in range(NT) for r in range(0, C, PR)]
        if CFG['BORD'] == 'rc':
            crs = [(c_, r) for r in range(0, C, PR) for c_ in range(NT)]
        for c_, r in crs:
            if True:
                re, im = slice(r, r + PR), slice(C + r, C + r + PR)
                L = lambda s_, sl: pool[s_, c_, sl, :]
                Y = lambda s_, sl: ypool[s_, c_, sl, :]
                u0r, u0i, u1r, u1i = L(us, re), L(us, im), L(us + 1, re), L(us + 1, im)
                kbr, kbi, kcr, kci = L(ks, re), L(ks, im), L(ks + 1, re), L(ks + 1, im)
                ar, ai = cmul(kbr, kbi, u0r, u0i)
                if not diag:
                    cr, ci = cmul(L(ks - 1, re), L(ks - 1, im), u1r, u1i)
                    ar, ai = ar + cr, ai + ci
                if CFG['FORM'] == 'seq':
                    if not first:
                        ar, ai = Y(ys, re) + ar, Y(ys, im) + ai
                    ypool[ys, c_, re, :] = ar
                    ypool[ys, c_, im, :] = ai
                br, bi = cmul(kcr, kci, u0r, u0i)
                dr, di = cmul(kbr, kbi, u1r, u1i)
                br, bi = br + dr, bi + di
                if not first:
                    br, bi = Y(ys + 1, re) + br, Y(ys + 1, im) + bi
                if CFG['FORM'] != 'seq':
                    if not first:
                        ar, ai = Y(ys, re) + ar, Y(ys, im) + ai
                    ypool[ys, c_, re, :] = ar
                    ypool[ys, c_, im, :] = ai
                ypool[ys + 1, c_, re, :] = br
                ypool[ys + 1, c_, im, :] = bi

    def sched_blocks(t):
        block(t, t, 0, True, False)
        for sched in _SCHED:
            I = (_pack([ij[0] for ij in sched]) >> (3 * t)) & 7
            J = (_pack([ij[1] for ij in sched]) >> (3 * t)) & 7
            block(I, J, I - J, False, False)

    def one_block(t, b):
        if b == 0:
            block(t, t, 0, True, False)
        else:
            sched = _SCHED[b - 1]
            I = (_pack([ij[0] for ij in sched]) >> (3 * t)) & 7
            J = (_pack([ij[1] for ij in sched]) >> (3 * t)) & 7
            block(I, J, I - J, False, False)

    def prep(t):
        if not CFG['USEPREP']:
            return
        slot = t % 2
        R = CFG['PREPR']
        for r in range(0, BM, R):
            x = q_s[pl.ds(pl.multiple_of(t * BM + r, R), R), :].astype(F32)
            gh = _layernorm(x) * bc(V_A1, R) + bc(V_SA, R)
            kv = get_kv(slot, r, R).astype(F32)
            gh_s[r:r + R, :] = gh
            x1_s[slot, r:r + R, :] = x + gh * (kv * bc(V_D, R))

    last_h2 = [None]

    def gate_k(t):
        z = last_h2[0][-HALO:, -128:]
        k_s[0:HALO, 0:128] = jnp.where(t < 0, z, 0.0).astype(BF16)

    def inverse_post(t, first=False):
        slot = t % 2
        for c in range(2):
            if first and c == 0:
                yf = get_y(0).astype(BF16)
            else:
                yf = (get_y(2 * t + c) + get_y(2 * t + c - 1)).astype(BF16)
            y = jnp.dot(pltpu.bitcast(g_s[2 * (t % 2) + c], BF16), yf, preferred_element_type=F32)
            R = CFG['POSTR']
            for r in range(0, C, R):
                rr = c * C + r
                if CFG['USEPREP']:
                    x1 = x1_s[slot, rr:rr + R, :] + gh_s[rr:rr + R, :] * y[r:r + R]
                else:
                    kv = get_kv(slot, rr, R).astype(F32)
                    yy = y[r:r + R] + kv * bc(V_D, R)
                    x = q_s[pl.ds(pl.multiple_of(t * BM + rr, R), R), :].astype(F32)
                    gh = _layernorm(x) * bc(V_A1, R) + bc(V_SA, R)
                    x1 = x + gh * yy
                x1_s[slot, rr:rr + R, :] = x1
                h2 = _layernorm(x1) * bc(V_B1, R) + bc(V_SB, R)
                last_h2[0] = h2
                if CFG['PACK']:
                    h2_s[slot, rr // 2:(rr + R) // 2, :] = pltpu.bitcast(h2.astype(BF16), jnp.uint32)
                else:
                    h2_s[slot, rr:rr + R, :] = h2.astype(BF16)

    def gate_up(t, j):
        h = pltpu.bitcast(h2_s[t % 2], BF16) if CFG['PACK'] else h2_s[t % 2]
        if not CFG['ILV']:
            g = jnp.dot(h, wgu_s[j, :, 0:FC], preferred_element_type=F32)
            u = jnp.dot(h, wgu_s[j, :, FC:2 * FC], preferred_element_type=F32)
            return (g * u).astype(BF16)
        gu = jnp.dot(h, wgu_s[j], preferred_element_type=F32)
        return jnp.concatenate([(gu[:, 2 * i * 128:(2 * i + 1) * 128] * gu[:, (2 * i + 1) * 128:(2 * i + 2) * 128]).astype(BF16)
                                for i in range(FC // 128)], axis=1)

    def put_hidden(j, a):
        a_s[:, j * FC:(j + 1) * FC] = pltpu.bitcast(a, jnp.uint32) if CFG['PACK'] else a

    def finish(t, o):
        o = x1_s[t % 2] + bc(V_GB, BM) * o
        out_s[pl.ds(pl.multiple_of(t * BM, BM), BM), :] = o.astype(BF16)
        cp_o(t).start()

    def down_out(t):
        a = pltpu.bitcast(a_s[...], BF16) if CFG['PACK'] else a_s[...]
        finish(t, jnp.dot(a, wd_s[...], preferred_element_type=F32))

    def mod(s, dst, plus_one):
        if s < 5:
            cp_wm(s).wait()
        m = jnp.dot(sc, wm_s[s], preferred_element_type=F32)[0:8]
        m = m.astype(BF16).astype(F32)
        vec[dst] = 1.0 + m if plus_one else m

    k_s[0:HALO, :] = jnp.zeros((HALO, D), BF16)
    for i in range(2 * _ZERO_FROM, 2 * NSTEP):
        ypool[yb + i] = jnp.zeros((NT, 2 * C, 128), F32)
    cp_small(0).wait()
    f_s[2:4] = f_s[0:2] ^ np.uint32(0x80008000)

    def k_piece(p, carry):
        cp_ssm(p).wait()

        @pl.when(p == 1)
        def _():
            for t in range(2):
                cp_k(t).start()
                cp_v(t).start()
            for s_ in range(2):
                cp_wm(s_).start()

        @pl.when(p == 3)
        def _():
            for s_ in range(2, 5):
                cp_wm(s_).start()
            cp_small(4).start()
            cp_q(0).start()
            cp_q(1).start()

        for i in range(SP // C):
            m = p * (SP // C) + i
            chunk = ssm_s[:, pl.ds(pl.multiple_of(m * C, C), C)]
            put_slot(KB + m, jax.lax.dot_general(pltpu.bitcast(f_s[i % 4], BF16), chunk, (((1,), (1,)), ((), ())),
                                                 preferred_element_type=F32))
        return carry

    jax.lax.fori_loop(0, NSP, k_piece, 0)

    for i in range(1, 4):
        cp_small(i).wait()
    sh = sh_s[...].astype(F32)
    for j in range(4):
        vec[V_W0 + j] = jnp.broadcast_to(sh[j:j + 1, :], (8, D))
    vec[V_D] = jnp.broadcast_to(d_s[...].astype(F32).reshape(1, D), (8, D))
    cf = c_s[...].astype(F32)
    sc = (cf * jax.nn.sigmoid(cf)).astype(BF16)
    sc = jnp.broadcast_to(sc, (16, D))

    def first_blocks(I, carry):
        block(I, 0, I, False, True)
        return carry

    def conv_step(t, carry):
        cp_k(t).wait()
        cp_v(t).wait()
        kv_fwd(t)

        @pl.when(t == 0)
        def _():
            for j in range(N1):
                cp_wg(j).start()
                cp_wu(j).start()
            block(0, 0, 0, True, True)
            jax.lax.fori_loop(1, _ZERO_FROM, first_blocks, 0)

        @pl.when(t == 1)
        def _():
            for j in range(NF):
                cp_wd(j).start()
            cp_wm(5).start()
            cp_k(2).start()
            cp_v(2).start()
            cp_q(2).start()
            block(t, t, 0, True, False)
            block(t + 1, t, 1, False, False)
        return carry

    jax.lax.fori_loop(0, 2, conv_step, 0)

    mod(0, V_SA, False)
    mod(1, V_A1, True)
    mod(2, V_GA, False)
    vec[V_A1] = vec[V_A1] * vec[V_GA]
    vec[V_SA] = vec[V_SA] * vec[V_GA]
    mod(3, V_SB, False)
    mod(4, V_B1, True)
    cp_small(4).wait()
    g_s[2:4] = g_s[0:2] ^ np.uint32(0x80008000)
    cp_q(0).wait()
    prep(0)
    inverse_post(0, True)
    cp_q(1).wait()
    prep(1)
    inverse_post(1)

    def mlp_first():
        h = pltpu.bitcast(h2_s[0], BF16) if CFG['PACK'] else h2_s[0]
        pending = []

        def flush():
            for col, val in pending:
                a_s[:, col:col + val.shape[1]] = pltpu.bitcast(val, jnp.uint32) if CFG['PACK'] else val
            pending.clear()

        for j in range(N1):
            cp_wg(j).wait()
            cp_wu(j).wait()
            flush()
            for jj, r, w in segments(j):
                g = jnp.dot(h, wgu_s[jj, :, r:r + w], preferred_element_type=F32)
                u = jnp.dot(h, wgu_s[jj, :, FC + r:FC + r + w], preferred_element_type=F32)
                pending.append((jj * FC + r, (g * u).astype(BF16)))
        for j in range(NF):
            cp_wd(j).wait()
        cp_k(3).start()
        cp_v(3).start()
        cp_q(3).start()
        flush()
        a = pltpu.bitcast(a_s[...], BF16) if CFG['PACK'] else a_s[...]
        o = jnp.dot(a, wd_s[...], preferred_element_type=F32)
        cp_wm(5).wait()
        mod(5, V_GB, False)
        finish(0, o)

    def mlp_last(t):
        for j in range(NF):
            put_hidden(j, gate_up(t, j))
        for hf in range(2):
            rows = slice(hf * C // 2, (hf + 1) * C // 2) if CFG['PACK'] else slice(hf * C, (hf + 1) * C)
            a = pltpu.bitcast(a_s[rows, :], BF16) if CFG['PACK'] else a_s[rows, :]
            o = jnp.dot(a, wd_s[...], preferred_element_type=F32)
            o = x1_s[t % 2, hf * C:(hf + 1) * C, :] + bc(V_GB, C) * o
            out_s[t * BM + hf * C:t * BM + (hf + 1) * C, :] = o.astype(BF16)
            cp_o_half(hf).start()

    def paired(t):
        u = t + 1
        cp_q(u).wait()
        if CFG['PIPE']:
            @pl.when(u < NSTEP - 1)
            def _():
                cp_k(u + 1).wait()
                cp_v(u + 1).wait()
        else:
            cp_k(u).wait()
            cp_v(u).wait()

        def starts():
            if CFG['PIPE']:
                @pl.when(jnp.logical_and(u >= 3, u < NSTEP - 1))
                def _():
                    cp_q(u + 1).start()

                @pl.when(u < NSTEP - 2)
                def _():
                    cp_k(u + 2).start()
                    cp_v(u + 2).start()
            else:
                @pl.when(jnp.logical_and(u >= 3, u < NSTEP - 1))
                def _():
                    cp_k(u + 1).start()
                    cp_v(u + 1).start()
                    cp_q(u + 1).start()

        gi = 0
        kv_u = None
        for ch in CFG['ORDER']:
            if ch == 'k':
                if CFG['PIPE']:
                    kv_u = None
                    make_kv(jnp.minimum(u + 1, NSTEP - 1), u + 1)
                else:
                    kv_u = make_kv(u)
            elif ch == 'G':
                gate_k(t)
            elif ch == 's':
                starts()
            elif ch == 'K':
                kv_fwd(u)
            elif ch == 'p':
                prep(u)
            elif ch == 'F':
                conv_fwd(u, kv_u)
            elif ch == 'P':
                sched_blocks(u)
            elif ch in '01234':
                one_block(u, int(ch))
            elif ch == 'g':
                put_hidden(gi, gate_up(t, gi))
                gi += 1
            elif ch == 'I':
                inverse_post(u)
            elif ch == 'd':
                down_out(t)

    mlp_first()
    if CFG['PIPE']:
        cp_k(2).wait()
        cp_v(2).wait()
        make_kv(2)
    jax.lax.fori_loop(1, NSTEP - 1, lambda t, c_: (paired(t), c_)[1], 0)
    mlp_last(NSTEP - 1)
    for t in range(NSTEP - 1):
        cp_o(t).wait()
    cp_o_half(0).wait()
    cp_o_half(1).wait()


@jax.jit
def pallas_adaLN_cond__ssm_conv_h3__glu_gated_bilinear__prompt_kernel(
    A_q: jax.Array,
    A_k: jax.Array,
    A_v: jax.Array,
    A_shift_k: jax.Array,
    A_ssm_k: jax.Array,
    A_ssm_D: jax.Array,
    B_x: jax.Array,
    B_w_gate: jax.Array,
    B_w_up: jax.Array,
    B_w_down: jax.Array,
    c: jax.Array,
    w_mod: jax.Array,
):
    del B_x
    fwd, inv = _dft_matrices()
    any_spec = pl.BlockSpec(memory_space=pl.ANY)
    scratch = [
        pltpu.VMEM((S, D), BF16),
        pltpu.VMEM((HALO + S, D), BF16),
        pltpu.VMEM((S, D), BF16),
        pltpu.VMEM((4, D), BF16),
        pltpu.VMEM((D, S), BF16),
        pltpu.VMEM((D,), BF16),
        pltpu.VMEM((NF, D, 2 * FC), BF16),
        pltpu.VMEM((FF, D), BF16),
        pltpu.VMEM((1, D), BF16),
        pltpu.VMEM((6, D, D), BF16),
        pltpu.VMEM((4, C, C), jnp.uint32),
        pltpu.VMEM((4, C // 2, 2 * C), jnp.uint32),
        pltpu.VMEM((34 if CFG['SPLIT'] else NSLOT, NT, 2 * C, 128), F32),
        pltpu.VMEM((16 if CFG['SPLIT'] else 1, NT, 2 * C, 128), F32),
        pltpu.VMEM((12, 8, D), F32),
        pltpu.VMEM((2, BM // 2, D), jnp.uint32) if CFG['PKV'] else pltpu.VMEM((2, BM, D), BF16),
        pltpu.VMEM((BM, D), F32),
        pltpu.VMEM((2, BM, D), F32),
        pltpu.VMEM((2, BM // 2, D), jnp.uint32) if CFG['PACK'] else pltpu.VMEM((2, BM, D), BF16),
        pltpu.VMEM((BM // 2, FF), jnp.uint32) if CFG['PACK'] else pltpu.VMEM((BM, FF), BF16),
        pltpu.VMEM((S, D), BF16),
        pltpu.SemaphoreType.DMA((5,)),
        pltpu.SemaphoreType.DMA((4,)),
        pltpu.SemaphoreType.DMA((6,)),
        pltpu.SemaphoreType.DMA((NSTEP,)),
        pltpu.SemaphoreType.DMA((NSTEP,)),
        pltpu.SemaphoreType.DMA((NSTEP,)),
        pltpu.SemaphoreType.DMA((FF // CFG['F1'],)),
        pltpu.SemaphoreType.DMA((FF // CFG['F1'],)),
        pltpu.SemaphoreType.DMA((FF // CFG['F1'],)),
        pltpu.SemaphoreType.DMA((NSTEP + 1,)),
    ]
    out = pl.pallas_call(
        _kernel,
        in_specs=[any_spec] * 13,
        out_specs=any_spec,
        out_shape=jax.ShapeDtypeStruct((S, D), BF16),
        scratch_shapes=scratch,
        compiler_params=pltpu.CompilerParams(vmem_limit_bytes=110 * 2**20, flags=FLAGS),
    )(A_q.reshape(S, D), A_k.reshape(S, D), A_v.reshape(S, D), A_shift_k.T, A_ssm_k, A_ssm_D,
      B_w_gate, B_w_up, B_w_down, c, w_mod, fwd, inv)
    return out.reshape(1, S, D)
```

```python
import numpy as np

import jax
import jax.numpy as jnp
import jax.experimental.pallas as pl
import jax.experimental.pallas.tpu as pltpu

S, D, FF = 2048, 640, 1536
C = 128
BM = 256
NSTEP = S // BM
NT = D // 128
HALO = 16
EPS = 1e-5

FC = 768
NF = FF // FC
FP = 512
NP = FF // FP
PR = 16
SP = 512
NSP = S // SP

KB, UB = 0, 16

F32, BF16 = jnp.float32, jnp.bfloat16

V_A1, V_SA, V_GA, V_B1, V_SB, V_GB, V_W0, V_D = 0, 1, 2, 3, 4, 5, 6, 10

_SCHED = [
    [(3, 1), (4, 2), (5, 2), (6, 1), (6, 5), (7, 3)],
    [(3, 2), (4, 3), (5, 3), (6, 2), (7, 0), (7, 4)],
    [(4, 0), (5, 0), (5, 4), (6, 3), (7, 1), (7, 5)],
    [(4, 1), (5, 1), (6, 0), (6, 4), (7, 2), (7, 6)],
]
_ZERO_FROM = 4


def _pack3(vals):
    r = 0
    for n, x in enumerate(vals):
        r |= x << (3 * (n + 2))
    return r


def _pack_rows(m):
    h = m.astype(np.float32).astype(BF16).view(np.uint16).astype(np.uint32)
    return h[:, 0::2, :] | (h[:, 1::2, :] << 16)


def _dft_matrices():
    f = np.arange(C, dtype=np.float64)[None, :, None] + 0.5
    s = np.arange(2 * C, dtype=np.float64).reshape(2, 1, C)
    ang = 2.0 * np.pi * f * s / (2 * C)
    fwd = np.concatenate([np.cos(ang), -np.sin(ang)], axis=1)
    inv = np.swapaxes(fwd, 1, 2) / C
    return _pack_rows(fwd), _pack_rows(inv)


def _layernorm(x):
    m = jnp.mean(x, axis=1, keepdims=True)
    xc = x - m
    v = jnp.mean(xc * xc, axis=1, keepdims=True)
    return xc * jax.lax.rsqrt(v + EPS)


def _pk(x):
    return pltpu.bitcast(x, jnp.uint32)


def _unpk(x):
    return pltpu.bitcast(x, BF16)


class _Copies:
    def __init__(self, copies):
        self.copies = copies

    def start(self):
        for c in self.copies:
            c.start()

    def wait(self):
        for c in self.copies:
            c.wait()


def _kernel(q_hbm, k_hbm, v_hbm, sh_hbm, ssm_hbm, d_hbm, wg_hbm, wu_hbm, wd_hbm, c_hbm, wm_hbm,
            f_hbm, g_hbm, o_hbm,
            q_s, k_s, v_s, sh_s, ssm_s, d_s, wgu_s, wd_s, c_s, wm_s, f_s, g_s,
            spec, acc, vec, kv_s, x1_s, h2_s, a_s, out_s,
            sem_small, sem_ssm, sem_wm, sem_k, sem_v, sem_q, sem_wg, sem_wu, sem_wd, sem_o):

    def cp_small(i):
        src, dst = [(f_hbm, f_s.at[0:2]), (sh_hbm, sh_s), (d_hbm, d_s), (c_hbm, c_s), (g_hbm, g_s.at[0:2])][i]
        return pltpu.make_async_copy(src, dst, sem_small.at[i])

    def cp_ssm(p):
        return pltpu.make_async_copy(ssm_hbm.at[:, pl.ds(p * SP, SP)], ssm_s.at[:, pl.ds(p * SP, SP)], sem_ssm.at[p])

    def cp_wm(s):
        return pltpu.make_async_copy(wm_hbm.at[:, pl.ds(s * D, D)], wm_s.at[s], sem_wm.at[s])

    def cp_k(t):
        return pltpu.make_async_copy(k_hbm.at[pl.ds(t * BM, BM)], k_s.at[pl.ds(HALO + t * BM, BM)], sem_k.at[t])

    def cp_v(t):
        return pltpu.make_async_copy(v_hbm.at[pl.ds(t * BM, BM)], v_s.at[pl.ds(t * BM, BM)], sem_v.at[t])

    def cp_q(t):
        return pltpu.make_async_copy(q_hbm.at[pl.ds(t * BM, BM)], q_s.at[pl.ds(t * BM, BM)], sem_q.at[t])

    def segments(j):
        out, lo = [], j * FP
        while lo < (j + 1) * FP:
            jj, r = divmod(lo, FC)
            w = min(FC - r, (j + 1) * FP - lo)
            out.append((jj, r, w))
            lo += w
        return out

    def cp_w(j, src, sem, off):
        return _Copies([pltpu.make_async_copy(src.at[:, pl.ds(jj * FC + r, w)],
                                              wgu_s.at[jj, :, pl.ds(off * FC + r, w)], sem.at[j])
                        for jj, r, w in segments(j)])

    def cp_wg(j):
        return cp_w(j, wg_hbm, sem_wg, 0)

    def cp_wu(j):
        return cp_w(j, wu_hbm, sem_wu, 1)

    def cp_wd(j):
        return pltpu.make_async_copy(wd_hbm.at[pl.ds(j * FC, FC)], wd_s.at[pl.ds(j * FC, FC)], sem_wd.at[j])

    def cp_o(t):
        return pltpu.make_async_copy(out_s.at[pl.ds(t * BM, BM)], o_hbm.at[pl.ds(t * BM, BM)], sem_o.at[t])

    def cp_o_last(half):
        r0 = (NSTEP - 1) * BM + half * C
        return pltpu.make_async_copy(out_s.at[pl.ds(r0, C)], o_hbm.at[pl.ds(r0, C)], sem_o.at[NSTEP - 1 + half])

    def start_step(t):
        cp_k(t).start()
        cp_v(t).start()
        cp_q(t).start()

    def bc(i, rows):
        return jnp.broadcast_to(vec[i, 0:1, :], (rows, D))

    def put_spec(slot, val):
        for c in range(NT):
            spec[slot, c] = val[:, c * 128:(c + 1) * 128]

    def get_acc(i):
        return jnp.concatenate([acc[i, c] for c in range(NT)], axis=1)

    def get_kv(t, c):
        return _unpk(kv_s[t % 2, c * C // 2:(c + 1) * C // 2, :])

    def kv_fwd(t):
        for c in range(2):
            r0 = pl.multiple_of(t * BM + c * C, C)
            kk = k_s[pl.ds(r0, C + HALO), :].astype(F32)
            ks = kk[HALO:] * bc(V_W0, C)
            for j in range(1, 4):
                ks = ks + kk[HALO - j:HALO - j + C] * bc(V_W0 + j, C)
            vv = v_s[pl.ds(r0, C), :].astype(F32)
            kv_s[t % 2, c * C // 2:(c + 1) * C // 2, :] = _pk((ks * vv).astype(BF16))
            u = jnp.dot(_unpk(f_s[2 * (t % 2) + c]), get_kv(t, c), preferred_element_type=F32)
            put_spec(UB + 2 * t + c, u)

    def cmul(kr, ki, ur, ui):
        return kr * ur - ki * ui, kr * ui + ki * ur

    def block(I, J, diag, first):
        ys, us, ks = 2 * I, UB + 2 * J, KB + 2 * (I - J)
        for c in range(NT):
            for r in range(0, C, PR):
                re, im = slice(r, r + PR), slice(C + r, C + r + PR)
                u0r, u0i = spec[us, c, re, :], spec[us, c, im, :]
                u1r, u1i = spec[us + 1, c, re, :], spec[us + 1, c, im, :]
                kbr, kbi = spec[ks, c, re, :], spec[ks, c, im, :]
                kcr, kci = spec[ks + 1, c, re, :], spec[ks + 1, c, im, :]
                ar, ai = cmul(kbr, kbi, u0r, u0i)
                if not diag:
                    cr, ci = cmul(spec[ks - 1, c, re, :], spec[ks - 1, c, im, :], u1r, u1i)
                    ar, ai = ar + cr, ai + ci
                br, bi = cmul(kcr, kci, u0r, u0i)
                dr, di = cmul(kbr, kbi, u1r, u1i)
                br, bi = br + dr, bi + di
                if not first:
                    br, bi = acc[ys + 1, c, re, :] + br, acc[ys + 1, c, im, :] + bi
                    ar, ai = acc[ys, c, re, :] + ar, acc[ys, c, im, :] + ai
                acc[ys, c, re, :] = ar
                acc[ys, c, im, :] = ai
                acc[ys + 1, c, re, :] = br
                acc[ys + 1, c, im, :] = bi

    def sched_blocks(t):
        block(t, t, True, False)
        for sched in _SCHED:
            I = (_pack3([ij[0] for ij in sched]) >> (3 * t)) & 7
            J = (_pack3([ij[1] for ij in sched]) >> (3 * t)) & 7
            block(I, J, False, False)

    def inverse_post(t, first=False):
        for c in range(2):
            if first and c == 0:
                yf = get_acc(0).astype(BF16)
            else:
                yf = (get_acc(2 * t + c) + get_acc(2 * t + c - 1)).astype(BF16)
            y = jnp.dot(_unpk(g_s[2 * (t % 2) + c]), yf, preferred_element_type=F32)
            yy = y + get_kv(t, c).astype(F32) * bc(V_D, C)
            x = q_s[pl.ds(pl.multiple_of(t * BM + c * C, C), C), :].astype(F32)
            gh = _layernorm(x) * bc(V_A1, C) + bc(V_SA, C)
            x1 = x + gh * yy
            x1_s[t % 2, c * C:(c + 1) * C, :] = x1
            h2 = _layernorm(x1) * bc(V_B1, C) + bc(V_SB, C)
            h2_s[t % 2, c * C // 2:(c + 1) * C // 2, :] = _pk(h2.astype(BF16))

    def hidden(h, jj, r, w):
        g = jnp.dot(h, wgu_s[jj, :, r:r + w], preferred_element_type=F32)
        u = jnp.dot(h, wgu_s[jj, :, FC + r:FC + r + w], preferred_element_type=F32)
        return (g * u).astype(BF16)

    def gate_up(t):
        for j in range(NF):
            a_s[:, j * FC:(j + 1) * FC] = _pk(hidden(_unpk(h2_s[t % 2]), j, 0, FC))

    def finish(t, o):
        o = x1_s[t % 2] + bc(V_GB, BM) * o
        out_s[pl.ds(pl.multiple_of(t * BM, BM), BM), :] = o.astype(BF16)
        cp_o(t).start()

    def mod(s, dst, plus_one):
        cp_wm(s).wait()
        m = jnp.dot(sc, wm_s[s], preferred_element_type=F32)[0:8]
        m = m.astype(BF16).astype(F32)
        vec[dst] = 1.0 + m if plus_one else m

    cp_small(0).start()
    cp_ssm(0).start()
    cp_ssm(1).start()
    for i in range(1, 4):
        cp_small(i).start()
    cp_ssm(2).start()
    cp_ssm(3).start()

    k_s[0:HALO, :] = jnp.zeros((HALO, D), BF16)
    for i in range(2 * _ZERO_FROM, 2 * NSTEP):
        acc[i] = jnp.zeros((NT, 2 * C, 128), F32)
    cp_small(0).wait()
    f_s[2:4] = f_s[0:2] ^ np.uint32(0x80008000)

    def k_piece(p, carry):
        cp_ssm(p).wait()

        @pl.when(p == 1)
        def _():
            for t in range(2):
                cp_k(t).start()
                cp_v(t).start()
            for s in range(2):
                cp_wm(s).start()

        @pl.when(p == NSP - 1)
        def _():
            for s in range(2, 5):
                cp_wm(s).start()
            cp_small(4).start()
            cp_q(0).start()
            cp_q(1).start()

        for i in range(SP // C):
            m = p * (SP // C) + i
            chunk = ssm_s[:, pl.ds(pl.multiple_of(m * C, C), C)]
            put_spec(KB + m, jax.lax.dot_general(_unpk(f_s[i % 4]), chunk, (((1,), (1,)), ((), ())),
                                                 preferred_element_type=F32))
        return carry

    jax.lax.fori_loop(0, NSP, k_piece, 0)

    for i in range(1, 4):
        cp_small(i).wait()
    sh = sh_s[...].astype(F32)
    for j in range(4):
        vec[V_W0 + j] = jnp.broadcast_to(sh[j:j + 1, :], (8, D))
    vec[V_D] = jnp.broadcast_to(d_s[...].astype(F32).reshape(1, D), (8, D))
    cf = c_s[...].astype(F32)
    sc = jnp.broadcast_to((cf * jax.nn.sigmoid(cf)).astype(BF16), (16, D))

    def first_blocks(I, carry):
        block(I, 0, False, True)
        return carry

    def conv_step(t, carry):
        cp_k(t).wait()
        cp_v(t).wait()
        kv_fwd(t)

        @pl.when(t == 0)
        def _():
            for j in range(NP):
                cp_wg(j).start()
                cp_wu(j).start()
            block(0, 0, True, True)
            jax.lax.fori_loop(1, _ZERO_FROM, first_blocks, 0)

        @pl.when(t == 1)
        def _():
            for j in range(NF):
                cp_wd(j).start()
            cp_wm(5).start()
            start_step(2)
            block(t, t, True, False)
            block(t + 1, t, False, False)
        return carry

    jax.lax.fori_loop(0, 2, conv_step, 0)

    mod(0, V_SA, False)
    mod(1, V_A1, True)
    mod(2, V_GA, False)
    vec[V_A1] = vec[V_A1] * vec[V_GA]
    vec[V_SA] = vec[V_SA] * vec[V_GA]
    mod(3, V_SB, False)
    mod(4, V_B1, True)
    cp_small(4).wait()
    cp_q(0).wait()
    g_s[2:4] = g_s[0:2] ^ np.uint32(0x80008000)
    inverse_post(0, True)
    cp_q(1).wait()
    inverse_post(1)

    h0 = _unpk(h2_s[0])
    pending = []

    def flush():
        for col, val in pending:
            a_s[:, col:col + val.shape[1]] = _pk(val)
        pending.clear()

    for j in range(NP):
        cp_wg(j).wait()
        cp_wu(j).wait()
        flush()
        for jj, r, w in segments(j):
            pending.append((jj * FC + r, hidden(h0, jj, r, w)))
    for j in range(NF):
        cp_wd(j).wait()
    start_step(3)
    flush()
    o0 = jnp.dot(_unpk(a_s[...]), wd_s[...], preferred_element_type=F32)
    mod(5, V_GB, False)
    finish(0, o0)

    def paired(t, carry):
        u = t + 1
        cp_q(u).wait()
        cp_k(u).wait()
        cp_v(u).wait()

        @pl.when(jnp.logical_and(u >= 3, u < NSTEP - 1))
        def _():
            start_step(u + 1)

        kv_fwd(u)
        sched_blocks(u)
        gate_up(t)
        inverse_post(u)
        finish(t, jnp.dot(_unpk(a_s[...]), wd_s[...], preferred_element_type=F32))
        return carry

    jax.lax.fori_loop(1, NSTEP - 1, paired, 0)

    t = NSTEP - 1
    gate_up(t)
    for half in range(2):
        o = jnp.dot(_unpk(a_s[half * C // 2:(half + 1) * C // 2, :]), wd_s[...], preferred_element_type=F32)
        o = x1_s[t % 2, half * C:(half + 1) * C, :] + bc(V_GB, C) * o
        out_s[t * BM + half * C:t * BM + (half + 1) * C, :] = o.astype(BF16)
        cp_o_last(half).start()

    for t in range(NSTEP - 1):
        cp_o(t).wait()
    cp_o_last(0).wait()
    cp_o_last(1).wait()


@jax.jit
def pallas_adaLN_cond__ssm_conv_h3__glu_gated_bilinear__prompt_kernel(
    A_q: jax.Array,
    A_k: jax.Array,
    A_v: jax.Array,
    A_shift_k: jax.Array,
    A_ssm_k: jax.Array,
    A_ssm_D: jax.Array,
    B_x: jax.Array,
    B_w_gate: jax.Array,
    B_w_up: jax.Array,
    B_w_down: jax.Array,
    c: jax.Array,
    w_mod: jax.Array,
):
    del B_x
    fwd, inv = _dft_matrices()
    any_spec = pl.BlockSpec(memory_space=pl.ANY)
    dma = pltpu.SemaphoreType.DMA
    scratch = [
        pltpu.VMEM((S, D), BF16),
        pltpu.VMEM((HALO + S, D), BF16),
        pltpu.VMEM((S, D), BF16),
        pltpu.VMEM((4, D), BF16),
        pltpu.VMEM((D, S), BF16),
        pltpu.VMEM((D,), BF16),
        pltpu.VMEM((NF, D, 2 * FC), BF16),
        pltpu.VMEM((FF, D), BF16),
        pltpu.VMEM((1, D), BF16),
        pltpu.VMEM((6, D, D), BF16),
        pltpu.VMEM((4, C, C), jnp.uint32),
        pltpu.VMEM((4, C // 2, 2 * C), jnp.uint32),
        pltpu.VMEM((32, NT, 2 * C, 128), F32),
        pltpu.VMEM((16, NT, 2 * C, 128), F32),
        pltpu.VMEM((11, 8, D), F32),
        pltpu.VMEM((2, BM // 2, D), jnp.uint32),
        pltpu.VMEM((2, BM, D), F32),
        pltpu.VMEM((2, BM // 2, D), jnp.uint32),
        pltpu.VMEM((BM // 2, FF), jnp.uint32),
        pltpu.VMEM((S, D), BF16),
        dma((5,)), dma((NSP,)), dma((6,)), dma((NSTEP,)), dma((NSTEP,)), dma((NSTEP,)),
        dma((NP,)), dma((NP,)), dma((NF,)), dma((NSTEP + 1,)),
    ]
    out = pl.pallas_call(
        _kernel,
        in_specs=[any_spec] * 13,
        out_specs=any_spec,
        out_shape=jax.ShapeDtypeStruct((S, D), BF16),
        scratch_shapes=scratch,
        compiler_params=pltpu.CompilerParams(vmem_limit_bytes=100 * 2**20),
    )(A_q.reshape(S, D), A_k.reshape(S, D), A_v.reshape(S, D), A_shift_k.T, A_ssm_k, A_ssm_D,
      B_w_gate, B_w_up, B_w_down, c, w_mod, fwd, inv)
    return out.reshape(1, S, D)
```
